```python
import os as _os
_os.environ.setdefault("JAX_PLATFORMS", "cpu")
import jax
import jax.numpy as jnp

def _softmax(x, axis=-1):
    return jax.nn.softmax(x, axis=axis)
def _gelu(x):
    return jax.nn.gelu(x, approximate=True)
def _silu(x):
    return jax.nn.silu(x)
def _sigmoid(x):
    return jax.nn.sigmoid(x)
def _layernorm(x, axis=-1, eps=1e-5):
    m = jnp.mean(x, axis=axis, keepdims=True)
    v = jnp.var(x, axis=axis, keepdims=True)
    return (x - m) / jnp.sqrt(v + eps)
def _scatter_add(tgt, idx, src, axis=0):
    return tgt.at[idx].add(src)
def _segment_sum(src, seg, n):
    return jax.ops.segment_sum(src, seg, n)
class _Rng:
    def __init__(self, key):
        self._k = key
    def _next(self):
        self._k, sub = jax.random.split(self._k)
        return sub
    def normal(self, shape):
        return jax.random.normal(self._next(), shape, dtype=jnp.bfloat16)
    def randint(self, lo, hi, shape):
        return jax.random.randint(self._next(), shape, lo, hi, dtype=jnp.int32)
    def uniform(self, shape, lo=0.0, hi=1.0):
        return jax.random.uniform(self._next(), shape, jnp.bfloat16, lo, hi)
    def permutation(self, n):
        return jax.random.permutation(self._next(), n)


kernel_name = 'gated_mix__softmax_full_mha__dense_activation_relu__prompt'

def setup_inputs():
    _rng = _Rng(jax.random.key(int.from_bytes(__import__("os").urandom(4), "little")))
    _w = (lambda a: (lambda t: t.astype(jnp.bfloat16) if jnp.issubdtype(t.dtype, jnp.floating) else t)(jnp.asarray(a)))
    def _A_setup():
        B, S, D = 1, 2048, 640
        return {
            "x": _w((lambda *s: _rng.normal(s) * 0.05)(B, S, D)),
            "wqkv": _w((lambda *s: _rng.normal(s) * 0.8)(D, 3 * D)),
            "wo": _w((lambda *s: _rng.normal(s) * 0.05)(D, D)),
        }
    _A_in = _A_setup()

    def _B_setup():
        B, S, D, Dff = 1, 2048, 640, 1536
        return {
            "x": _w((lambda *s: _rng.normal(s) * 0.05)(B, S, D)),
            "w1": _w((lambda *s: _rng.normal(s) * 0.05)(D, Dff)),
            "w2": _w((lambda *s: _rng.normal(s) * 0.05)(Dff, D)),
        }
    _B_in = _B_setup()

    return {
        "A_x": _A_in["x"],
        "A_wqkv": _A_in["wqkv"],
        "A_wo": _A_in["wo"],
        "B_x": _B_in["x"],
        "B_w1": _B_in["w1"],
        "B_w2": _B_in["w2"],
        "gate_w": _w((lambda *s: _rng.normal(s) * 0.05)(640) * 16.0),
    }

def reference(A_x, A_wqkv, A_wo, B_x, B_w1, B_w2, gate_w):
    def _A_ref(x, wqkv, wo):
        B, S, D = x.shape
        H = 32; Dh = D // H
        qkv = (lambda x, *d: x.transpose(*d))((x @ wqkv).reshape(B, S, 3, H, Dh), 2, 0, 3, 1, 4)
        q, k, v = qkv[0], qkv[1], qkv[2]
        scale = Dh ** -0.5
        scores = jnp.einsum("bhqd,bhkd->bhqk", q, k) * scale
        p = _softmax(scores, axis=-1)
        o = jnp.einsum("bhqk,bhkd->bhqd", p, v)
        return (lambda x, *d: x.transpose(*d))(o, 0, 2, 1, 3).reshape(B, S, D) @ wo

    def _B_ref(x, w1, w2):
        h = jnp.einsum("bsd,df->bsf", x, w1)
        zero = jnp.zeros_like(h)
        h = jnp.maximum(h, zero)
        return jnp.einsum("bsf,fd->bsd", h, w2)

    x = A_x
    g = _sigmoid((x * gate_w).sum(-1, keepdims=True))
    a = _A_ref(x, A_wqkv, A_wo)
    b = _B_ref(x, B_w1, B_w2)
    return g * a + (1 - g) * b
```

```python
import functools
import math
import jax
import jax.numpy as jnp
from jax import lax
import jax.experimental.pallas as pl
import jax.experimental.pallas.tpu as pltpu

S = 2048
D = 640
H = 32
DH = 20
DFF = 1536
HPG = 6
NG = 6
VR = 24
ONE_LANE = 120
TQ = 512
TK = 256
QSCALE = (DH ** -0.5) * math.log2(math.e)
L_MIN = 2.0 ** -40
F32 = jnp.float32
BF16 = jnp.bfloat16
NT = (((1,), (1,)), ((), ()))


def _kernel(x_ref, wk_ref, wqv_ref, wo_ref, w1_ref, w2_ref, gw_ref, o_ref,
            k_scr, qt_scr, vt_scr, ot_scr, nb_scr, lmin_scr):
    RC = 512
    lane = lax.broadcasted_iota(jnp.int32, (RC, 128), 1)
    rowv = lax.broadcasted_iota(jnp.int32, (NG * 128, RC), 0)
    er = lax.broadcasted_iota(jnp.int32, (H, NG * 128), 0)
    ec = lax.broadcasted_iota(jnp.int32, (H, NG * 128), 1)
    lo = (er // HPG) * 128 + (er % HPG) * DH
    e_ind = jnp.where((ec >= lo) & (ec < lo + DH), 1.0, 0.0).astype(BF16)

    kn_max = jnp.zeros((H, 128), F32)
    qn_parts = []
    for r in range(S // RC):
        xr = x_ref[r * RC:(r + 1) * RC, :]
        k = jnp.dot(xr, wk_ref[...], preferred_element_type=F32)
        kb = k.astype(BF16)
        kf = kb.astype(F32)
        kk = (kf * kf).astype(BF16)
        kn = lax.dot_general(e_ind, kk, NT, preferred_element_type=F32)
        for j in range(RC // 128):
            kn_max = jnp.maximum(kn_max, kn[:, j * 128:(j + 1) * 128])
        for g in range(NG):
            kg = k[:, g * 128:(g + 1) * 128]
            k_scr[g, r * RC:(r + 1) * RC, :] = jnp.where(lane == ONE_LANE, 1.0, kg).astype(BF16)
        qv = lax.dot_general(wqv_ref[...], xr, NT, preferred_element_type=F32)
        q = (qv[:NG * 128] * QSCALE).astype(BF16).astype(F32)
        qt_scr[:, r * RC:(r + 1) * RC] = q
        qn = jnp.dot(e_ind, (q * q).astype(BF16), preferred_element_type=F32)
        qn_parts.append(qn)
        v = qv[NG * 128:].astype(BF16).astype(F32)
        vt_scr[:, r * RC:(r + 1) * RC] = jnp.where(rowv % VR == DH, 1.0, v)
    kn_col = jnp.max(kn_max, axis=1, keepdims=True)
    for r in range(S // RC):
        nb_scr[:, r * RC:(r + 1) * RC] = -(jnp.sqrt(qn_parts[r] * kn_col) * 1.02)
    lmin_scr[...] = jnp.full(lmin_scr.shape, jnp.inf, F32)

    rowq = lax.broadcasted_iota(jnp.int32, (128, TQ), 0)
    NQ = S // TQ
    NC = S // TK

    def head_setup(h):
        g = h // HPG
        j = h - g * HPG
        return g, j * DH, pl.multiple_of(g * 128, 128), pl.multiple_of(h * VR, 8)

    def finish(h, v0, qi, acc):
        l = acc[DH:DH + 1, :]
        lmin_scr[:, qi * TQ:(qi + 1) * TQ] = jnp.minimum(lmin_scr[:, qi * TQ:(qi + 1) * TQ], l)
        ot_scr[pl.ds(v0, VR), qi * TQ:(qi + 1) * TQ] = acc * (1.0 / l)

    def fast_head(h, carry):
        g, r0, q0, v0 = head_setup(h)
        steps = [(qi, c) for qi in range(NQ) for c in range(NC)]
        lag = 1
        ps, accs, qms = {}, {}, {}
        for t in range(len(steps) + lag):
            if t < len(steps):
                qi, c = steps[t]
                if qi not in qms:
                    qg = qt_scr[pl.ds(q0, 128), qi * TQ:(qi + 1) * TQ]
                    nb = nb_scr[pl.ds(h, 1), qi * TQ:(qi + 1) * TQ]
                    qm = jnp.where((rowq >= r0) & (rowq < r0 + DH), qg, 0.0)
                    qm = jnp.where(rowq == ONE_LANE, nb, qm)
                    qms[qi] = qm.astype(BF16)
                s = jnp.dot(k_scr[g, c * TK:(c + 1) * TK, :], qms[qi], preferred_element_type=F32)
                ps[t] = jnp.exp2(s)
            if t - lag >= 0:
                qi, c = steps[t - lag]
                d = jnp.dot(vt_scr[pl.ds(v0, VR), c * TK:(c + 1) * TK], ps.pop(t - lag),
                            preferred_element_type=F32)
                accs[qi] = d if qi not in accs else accs[qi] + d
                if c == NC - 1:
                    finish(h, v0, qi, accs.pop(qi))
        return carry

    lax.fori_loop(0, H, fast_head, 0)

    safe = jnp.min(lmin_scr[...]) >= L_MIN

    @pl.when(jnp.logical_not(safe))
    def _():
        def slow_tile(it, carry):
            h = it // NQ
            qi = it - h * NQ
            g, r0, q0, v0 = head_setup(h)
            c0 = pl.multiple_of(qi * TQ, TQ)
            qg = qt_scr[pl.ds(q0, 128), pl.ds(c0, TQ)]
            qm = jnp.where((rowq >= r0) & (rowq < r0 + DH), qg, 0.0).astype(BF16)
            s = jnp.dot(k_scr[g], qm, preferred_element_type=F32)
            m = jnp.max(s, axis=0, keepdims=True)
            p = jnp.exp2(s - m)
            acc = jnp.dot(vt_scr[pl.ds(v0, VR), :], p, preferred_element_type=F32)
            ot_scr[pl.ds(v0, VR), pl.ds(c0, TQ)] = acc * (1.0 / acc[DH:DH + 1, :])
            return carry
        lax.fori_loop(0, H * NQ, slow_tile, 0)

    gw = gw_ref[...].astype(F32)
    for r in range(S // RC):
        xr = x_ref[r * RC:(r + 1) * RC, :]
        at = jnp.dot(wo_ref[...], ot_scr[:, r * RC:(r + 1) * RC].astype(BF16),
                     preferred_element_type=F32)
        a = at.T
        hh = jnp.maximum(jnp.dot(xr, w1_ref[...], preferred_element_type=F32), 0.0).astype(BF16)
        b = jnp.dot(hh, w2_ref[...], preferred_element_type=F32)
        z = jnp.sum(xr.astype(F32) * gw, axis=1, keepdims=True)
        gt = 1.0 / (1.0 + jnp.exp(-z))
        o_ref[r * RC:(r + 1) * RC, :] = (gt * a + (1.0 - gt) * b).astype(o_ref.dtype)


def _group_cols(w):
    w = jnp.pad(w, ((0, 0), (0, NG * HPG * DH - D))).reshape(D, NG, HPG * DH)
    return jnp.pad(w, ((0, 0), (0, 0), (0, 128 - HPG * DH))).reshape(D, NG * 128)


def _pad_heads(w):
    return jnp.pad(w.reshape(D, H, DH), ((0, 0), (0, 0), (0, VR - DH))).reshape(D, H * VR)


@jax.jit
def pallas_gated_mix__softmax_full_mha__dense_activation_relu__prompt_kernel(A_x, A_wqkv, A_wo, B_x, B_w1, B_w2, gate_w):
    x = A_x.reshape(S, D)
    wk = _group_cols(A_wqkv[:, D:2 * D])
    wqv = jnp.concatenate([_group_cols(A_wqkv[:, :D]), _pad_heads(A_wqkv[:, 2 * D:])], axis=1).T
    wo = _pad_heads(A_wo.T)
    gw = gate_w.reshape(1, D)
    out = pl.pallas_call(
        _kernel,
        out_shape=jax.ShapeDtypeStruct((S, D), A_x.dtype),
        scratch_shapes=[
            pltpu.VMEM((NG, S, 128), BF16),
            pltpu.VMEM((NG * 128, S), F32),
            pltpu.VMEM((H * VR, S), F32),
            pltpu.VMEM((H * VR, S), F32),
            pltpu.VMEM((H, S), F32),
            pltpu.VMEM((1, S), F32),
        ],
        compiler_params=pltpu.CompilerParams(vmem_limit_bytes=100 * 1024 * 1024),
    )(x, wk, wqv, wo, B_w1, B_w2, gw)
    return out.reshape(1, S, D)
```

```python
import functools
import math
import jax
import jax.numpy as jnp
from jax import lax
import jax.experimental.pallas as pl
import jax.experimental.pallas.tpu as pltpu

_cfg = dict(XR=32, R=4, G=5, LK=1, FS=6, FO=2, NTRIP=16, PPI=1, XST=1, KXS=0, QMS=0)

S = 2048
D = 640
H = 32
DH = 20
DFF = 1536
NP = H // 2
PR = 2 * DH
PPG = 3
NG = 6
ONE_LANE = 120
TQ = 512
TK = 256
RC = 512
NRC = S // RC
QSCALE = (DH ** -0.5) * math.log2(math.e)
L_MIN = 2.0 ** -40
F32 = jnp.float32
BF16 = jnp.bfloat16
NT = (((1,), (1,)), ((), ()))
NQ = S // TQ
NC = S // TK
CT = TQ // 128
FT = S // NP
XR = _cfg['XR']; R = _cfg['R']; G = _cfg['G']; LK = _cfg['LK']; PPI = _cfg['PPI']
XK = XR * NC
OUT_CHUNKS = [(0, 512), (512, 1024), (1024, 1536), (1536, 1920), (1920, 2048)]


def _kernel(x_hbm, wqkv_hbm, wo_hbm, w1_hbm, w2_hbm, gw_hbm, o_hbm,
            x_v, wqkv_v, wo_v, w1_v, w2_v, gw_v, o_v,
            wkp_scr, wqvt_scr, k_scr, qt_scr, vt_scr, ot_scr, lmin_scr, bb_scr, g_scr,
            kb0, kb1, qh0, qh1, kst, vst, xst, kxs, sems):
    cp_wk = pltpu.make_async_copy(wqkv_hbm.at[:, D:2 * D], wqkv_v.at[:, D:2 * D], sems.at[0])
    cp_x = [pltpu.make_async_copy(x_hbm.at[0, r * RC:(r + 1) * RC, :], x_v.at[r * RC:(r + 1) * RC, :],
                                  sems.at[1 + r]) for r in range(NRC)]
    cp_wq = pltpu.make_async_copy(wqkv_hbm.at[:, 0:D], wqkv_v.at[:, 0:D], sems.at[5])
    cp_wv = pltpu.make_async_copy(wqkv_hbm.at[:, 2 * D:], wqkv_v.at[:, 2 * D:], sems.at[6])
    cp_w1 = pltpu.make_async_copy(w1_hbm, w1_v, sems.at[7])
    cp_w2 = pltpu.make_async_copy(w2_hbm, w2_v, sems.at[8])
    cp_wo = pltpu.make_async_copy(wo_hbm, wo_v, sems.at[9])
    cp_gw = pltpu.make_async_copy(gw_hbm, gw_v, sems.at[10])
    cp_out = [pltpu.make_async_copy(o_v.at[r0:r1, :], o_hbm.at[0, r0:r1, :], sems.at[11 + i])
              for i, (r0, r1) in enumerate(OUT_CHUNKS)]
    cp_wk.start()
    cp_x[0].start()

    cp_wk.wait()
    cp_x[0].wait()
    cp_x[1].start()
    cp_x[2].start()
    GW = PPG * PR
    for rb in range(D // 128):
        wk = wqkv_v[rb * 128:(rb + 1) * 128, D:2 * D].astype(F32)
        for g in range(NG):
            n = min(GW, D - g * GW)
            piece = jnp.concatenate([wk[:, g * GW:g * GW + n], jnp.zeros((128, 128 - n), F32)], axis=1)
            wkp_scr[rb * 128:(rb + 1) * 128, g * 128:(g + 1) * 128] = piece.astype(BF16)

    lane = lax.broadcasted_iota(jnp.int32, (RC, 128), 1)
    er = lax.broadcasted_iota(jnp.int32, (16, 128), 0)
    ec = lax.broadcasted_iota(jnp.int32, (16, 128), 1)
    e_k = jnp.where((ec >= er * DH) & (ec < er * DH + DH) & (er < 2 * PPG), 1.0, 0.0).astype(BF16)
    kn_max = [None] * NG

    def k_norm(r, g):
        kf = k_scr[g, r * RC:(r + 1) * RC, :].astype(F32)
        kn = lax.dot_general(e_k, (kf * kf).astype(BF16), NT, preferred_element_type=F32)[0:8]
        kn_max[g] = kn if kn_max[g] is None else jnp.maximum(kn_max[g], kn)

    def k_proj(r):
        xr = x_v[r * RC:(r + 1) * RC, :]
        for g2 in range(NG // 2):
            k = jnp.dot(xr, wkp_scr[:, g2 * 256:(g2 + 1) * 256], preferred_element_type=F32)
            for g in (2 * g2, 2 * g2 + 1):
                kg = k[:, (g % 2) * 128:(g % 2 + 1) * 128]
                k_scr[g, r * RC:(r + 1) * RC, :] = jnp.where(lane == ONE_LANE, 1.0, kg).astype(BF16)
                if r > 0:
                    k_norm(r - 1, g)

    k_proj(0)
    cp_x[1].wait()
    cp_x[2].wait()
    for cp in (cp_x[3], cp_wv, cp_wq):
        cp.start()
    k_proj(1)
    k_proj(2)
    for cp in (cp_x[3], cp_wv, cp_wq):
        cp.wait()
    for cp in (cp_w1, cp_w2, cp_wo, cp_gw):
        cp.start()
    for cb in range(2 * D // 128):
        src_col = (2 * D if cb < D // 128 else -D) + cb * 128
        wqvt_scr[cb * 128:(cb + 1) * 128, :] = (
            wqkv_v[:, src_col:src_col + 128].astype(F32).T.astype(BF16))
    k_proj(3)

    for r in range(NRC):
        xr = x_v[r * RC:(r + 1) * RC, :]
        cols = slice(r * RC, (r + 1) * RC)
        for half in range(2):
            rows = slice(half * (D // 2), (half + 1) * (D // 2))
            v = lax.dot_general(wqvt_scr[rows, :], xr, NT, preferred_element_type=F32)
            vt_scr[rows, cols] = v.astype(BF16).astype(F32)
            if 2 * r + half < NG:
                k_norm(NRC - 1, 2 * r + half)
    kn_rows = [jnp.max(kn_max[g], axis=1, keepdims=True) for g in range(NG)]
    er = lax.broadcasted_iota(jnp.int32, (H, D), 0)
    ec = lax.broadcasted_iota(jnp.int32, (H, D), 1)
    e_q = jnp.where((ec >= er * DH) & (ec < er * DH + DH), 1.0, 0.0).astype(BF16)
    kn_col = jnp.concatenate([kn_rows[g][0:min(2 * PPG, H - 2 * PPG * g)] for g in range(NG)], axis=0)
    opaque0 = jnp.clip(-(jnp.minimum(jnp.min(kn_col), 0.0).astype(jnp.int32)), 0, DH * XK // 8)
    fence_row = pl.multiple_of((DH * XK // 8 - opaque0) * 8, 8)

    for r in range(NRC):
        xr = x_v[r * RC:(r + 1) * RC, :]
        cols = slice(r * RC, (r + 1) * RC)
        q = lax.dot_general(wqvt_scr[D:, :], xr, NT, preferred_element_type=F32)
        q = (q * QSCALE).astype(BF16).astype(F32)
        qn = jnp.dot(e_q, (q * q).astype(BF16), preferred_element_type=F32)
        nb = -(jnp.sqrt(qn * kn_col) * 1.02)
        nb = nb.astype(BF16).astype(F32)
        for p in range(NP):
            qt_scr[p, 0:PR, cols] = q[p * PR:(p + 1) * PR]
            nbt = nb[8 * (p // 4):8 * (p // 4) + 8]
            if p % 4:
                nbt = pltpu.roll(nbt, 8 - 2 * (p % 4), axis=0)
            qt_scr[p, PR:PR + 8, cols] = nbt
    lmin_scr[...] = jnp.full(lmin_scr.shape, jnp.inf, F32)

    sub_q = lax.broadcasted_iota(jnp.int32, (8, TQ), 0)
    kbs = (kb0, kb1)
    qhs = (qh0, qh1)

    def make_qm(q, nb, pos, hb):
        z8 = jnp.zeros((8, TQ), F32)
        if hb == 0:
            piece = [q[0:16], jnp.where(sub_q < 4, q[16:24], 0.0), z8, z8]
        else:
            piece = [z8, z8, jnp.where(sub_q >= 4, q[0:8], 0.0), q[8:24]]
        rows = []
        for pp in range(PPG):
            rows += [jnp.where(pos == pp, a, jnp.zeros_like(a)) for a in piece]
        rows.append(z8 if nb is None else jnp.where(sub_q == 0, nb, 0.0))
        return jnp.concatenate(rows, axis=0).astype(BF16)

    def v_lhs(r0, hb):
        sub = lax.broadcasted_iota(jnp.int32, (8, S), 0)
        v = vt_scr[pl.ds(r0 + 16 * hb, 24), :]
        if hb == 0:
            return jnp.concatenate([v[0:16], jnp.where(sub == 4, 1.0, v[16:24])], axis=0)
        return jnp.concatenate([jnp.where(sub == 3, 1.0, v[0:8]), v[8:24]], axis=0)

    def write_o(r0, hb, cols, acc):
        lrow = 20 if hb == 0 else 3
        l = acc[lrow:lrow + 1, :]
        o = acc * (1.0 / l)
        if hb == 0:
            ot_scr[pl.ds(r0, 24), cols] = o
        else:
            mid = ot_scr[pl.ds(r0 + 16, 8), cols]
            ot_scr[pl.ds(r0 + 16, 24), cols] = jnp.concatenate(
                [jnp.where(sub_q < 4, mid, o[0:8]), o[8:24]], axis=0)
        return l

    def pair_setup(p):
        g = p // PPG
        return g, p - g * PPG, pl.multiple_of(p * PR, 8)

    def stage_kx(p):
        g, pos, _ = pair_setup(p)
        for c in range(NC):
            kx = k_scr[g, c * TK:c * TK + XR, :].astype(F32)
            kxs[c * XR:(c + 1) * XR, :] = pltpu.roll(kx, (128 - pos * PR) % 128, axis=1).astype(kxs.dtype)

    def build_kb(hb, c, d0, d1, p=0):
        if _cfg['KXS']:
            kx = kxs[c * XR:(c + 1) * XR, :].astype(F32)
        else:
            g, pos, _ = pair_setup(p)
            kx = k_scr[g, c * TK:c * TK + XR, :].astype(F32)
            kx = pltpu.roll(kx, (128 - pos * PR) % 128, axis=1)
        for d in range(d0, d1):
            col = hb * DH + d
            kbs[hb][d * XK + c * XR:d * XK + (c + 1) * XR, :] = jnp.broadcast_to(kx[:, col:col + 1], (XR, 128))

    def build_qh(p, hb, qi):
        cols = slice(qi * TQ, (qi + 1) * TQ)
        qhs[hb][0:24, cols] = qt_scr[p, 16 * hb:16 * hb + 24, cols]
        qhs[hb][24:32, cols] = qt_scr[p, PR:PR + 8, cols]

    stage_kx(0)
    for c in range(NC):
        build_kb(0, c, 0, DH)
    for qi in range(NQ):
        build_qh(0, 0, qi)

    for cp in (cp_w1, cp_w2, cp_wo, cp_gw):
        cp.wait()
    gw = gw_v[...].astype(F32)

    def ffn_pieces(rows):
        if _cfg['XST']:
            xst[...] = x_v[rows, :]
        xsrc = (lambda: xst[...]) if _cfg['XST'] else (lambda: x_v[rows, :])
        hs = []
        for n in range(DFF // 256):
            hs.append(jnp.maximum(jnp.dot(xsrc(), w1_v[:, n * 256:(n + 1) * 256], preferred_element_type=F32),
                                  0.0).astype(BF16))
            yield
        hh = jnp.concatenate(hs, axis=1)
        z = jnp.sum(xsrc().astype(F32) * gw, axis=1, keepdims=True)
        gt = 1.0 / (1.0 + jnp.exp(-z))
        g_scr[rows, :] = jnp.broadcast_to(gt, (gt.shape[0], 128))
        for n in range(D // 128):
            b = jnp.dot(hh, w2_v[:, n * 128:(n + 1) * 128], preferred_element_type=F32)
            bb_scr[rows, n * 128:(n + 1) * 128] = (1.0 - gt) * b
            yield

    def fast_pairs(it, carry):
        hist = []

        def fence(hb):
            if not hist:
                return
            vals = [a[8 * i:8 * i + 8] for a in hist[-1] for i in range(R)]
            while len(vals) > 1:
                vals = [jnp.maximum(vals[2 * k], vals[2 * k + 1]) for k in range(len(vals) // 2)]
            kbs[hb][pl.ds(fence_row, 8), :] = vals[0]

        def vpu_block(hb, qi, row0):
            accs = []
            for d in range(DH):
                if d % G == 0:
                    fence(hb)
                if d == 0:
                    for c in range(CT):
                        col = qi * TQ + c * 128
                        accs.append(jnp.broadcast_to(qhs[hb][24 + hb:25 + hb, col:col + 128], (8 * R, 128)))
                kb = kbs[hb][d * XK + row0:d * XK + row0 + 8 * R, :]
                for c in range(CT):
                    col = qi * TQ + c * 128
                    qb = jnp.broadcast_to(qhs[hb][4 * hb + d:4 * hb + d + 1, col:col + 128], (8 * R, 128))
                    accs[c] = accs[c] + kb * qb
                if d % G == G - 1 - LK:
                    hist.append(list(accs))
            return jnp.concatenate(accs, axis=1)

        steps = [(j, hb, qi, c) for j in range(PPI) for hb in range(2) for qi in range(NQ) for c in range(NC)]
        ps, accs, qms = {}, {}, {}
        ffn = iter(())
        for t in range(len(steps) + 1):
            if t < len(steps):
                j, hb, qi, c = steps[t]
                p = it * PPI + j
                g, pos, r0 = pair_setup(p)
                pn = jnp.minimum(p + 1, NP - 1)
                cols = slice(qi * TQ, (qi + 1) * TQ)
                if (hb, qi, c) == (0, 0, 0):
                    kst[j] = k_scr[g]
                    for hh in range(2):
                        vst[j, hh] = v_lhs(r0, hh)
                    for _ in ffn:
                        pass
                    ffn = ffn_pieces(pl.ds(pl.multiple_of(p * FT, FT), FT))
                if (hb, qi, c) == (1, 0, 0) and _cfg['KXS']:
                    stage_kx(pn)
                if c == 0:
                    qms[(j, hb, qi)] = make_qm(qhs[hb][0:24, cols], qhs[hb][24 + hb:25 + hb, cols], pos, hb) if _cfg['QMS'] else make_qm(qt_scr[p, 16 * hb:16 * hb + 24, cols], qt_scr[p, PR + hb:PR + hb + 1, cols], pos, hb)
                s = jnp.dot(kst[j, c * TK + XR:(c + 1) * TK, :], qms[(j, hb, qi)], preferred_element_type=F32)
                sv = [vpu_block(hb, qi, c * XR + b * 8 * R) for b in range(XR // (8 * R))]
                build_kb(1 - hb, c, qi * DH // NQ, (qi + 1) * DH // NQ, p if hb == 0 else pn)
                if c == 0:
                    build_qh(p if hb == 0 else pn, 1 - hb, qi)
                ps[t] = jnp.exp2(jnp.concatenate(sv + [s], axis=0))
            if t >= 1:
                j, hb, qi, c = steps[t - 1]
                _, _, r0 = pair_setup(it * PPI + j)
                d = jnp.dot(vst[j, hb, :, c * TK:(c + 1) * TK], ps.pop(t - 1), preferred_element_type=F32)
                key = (j, hb, qi)
                accs[key] = d if key not in accs else accs[key] + d
                if c == NC - 1:
                    cols = slice(qi * TQ, (qi + 1) * TQ)
                    l = write_o(r0, hb, cols, accs.pop(key))
                    lmin_scr[:, cols] = jnp.minimum(lmin_scr[:, cols], l)
            if t % _cfg['FS'] == _cfg['FO']:
                next(ffn, None)
        for _ in ffn:
            pass
        return carry

    lax.fori_loop(0, _cfg['NTRIP'] // PPI, fast_pairs, 0)

    safe = jnp.min(lmin_scr[...]) >= L_MIN

    @pl.when(jnp.logical_not(safe))
    def _():
        def slow_tile(it, carry):
            p = it // NQ
            qi = it - p * NQ
            g, pos, r0 = pair_setup(p)
            cols = pl.ds(pl.multiple_of(qi * TQ, TQ), TQ)
            for hb in range(2):
                qm = make_qm(qt_scr[p, 16 * hb:16 * hb + 24, cols], None, pos, hb)
                s = jnp.dot(k_scr[g], qm, preferred_element_type=F32)
                m = jnp.max(s, axis=0, keepdims=True)
                pr = jnp.exp2(s - m)
                acc = jnp.dot(v_lhs(r0, hb), pr, preferred_element_type=F32)
                write_o(r0, hb, cols, acc)
            return carry
        lax.fori_loop(0, NP * NQ, slow_tile, 0)

    for i, (r0, r1) in enumerate(OUT_CHUNKS):
        rows = slice(r0, r1)
        o = ot_scr[:, rows].T.astype(BF16)
        a = jnp.dot(o, wo_v[...], preferred_element_type=F32)
        gt = g_scr[rows, :]
        for n in range(D // 128):
            cs = slice(n * 128, (n + 1) * 128)
            o_v[rows, cs] = (gt * a[:, cs] + bb_scr[rows, cs]).astype(o_v.dtype)
        cp_out[i].start()
    for cp in cp_out:
        cp.wait()


@jax.jit
def pallas_gated_mix__softmax_full_mha__dense_activation_relu__prompt_kernel(
        A_x, A_wqkv, A_wo, B_x, B_w1, B_w2, gate_w):
    gw = gate_w.reshape(1, D)
    return pl.pallas_call(
        _kernel,
        in_specs=[pl.BlockSpec(memory_space=pl.ANY)] * 6,
        out_specs=pl.BlockSpec(memory_space=pl.ANY),
        out_shape=jax.ShapeDtypeStruct((1, S, D), A_x.dtype),
        scratch_shapes=[
            pltpu.VMEM((S, D), BF16),
            pltpu.VMEM((D, 3 * D), BF16),
            pltpu.VMEM((D, D), BF16),
            pltpu.VMEM((D, DFF), BF16),
            pltpu.VMEM((DFF, D), BF16),
            pltpu.VMEM((1, D), BF16),
            pltpu.VMEM((S, D), BF16),
            pltpu.VMEM((D, NG * 128), BF16),
            pltpu.VMEM((2 * D, D), BF16),
            pltpu.VMEM((NG, S, 128), BF16),
            pltpu.VMEM((NP, PR + 8, S), F32),
            pltpu.VMEM((D, S), F32),
            pltpu.VMEM((D, S), F32),
            pltpu.VMEM((1, S), F32),
            pltpu.VMEM((S, D), F32),
            pltpu.VMEM((S, 128), F32),
            pltpu.VMEM((DH * XK + 8, 128), F32),
            pltpu.VMEM((DH * XK + 8, 128), F32),
            pltpu.VMEM((32, S), F32),
            pltpu.VMEM((32, S), F32),
            pltpu.VMEM((PPI, S, 128), BF16),
            pltpu.VMEM((PPI, 2, 24, S), F32),
            pltpu.VMEM((FT, D), BF16),
            pltpu.VMEM((XK, 128), BF16 if _cfg['KXS'] == 2 else F32),
            pltpu.SemaphoreType.DMA((11 + len(OUT_CHUNKS),)),
        ],
        compiler_params=pltpu.CompilerParams(vmem_limit_bytes=100 * 1024 * 1024),
    )(A_x, A_wqkv, A_wo, B_w1, B_w2, gw)
```

```python
import functools
import math
import jax
import jax.numpy as jnp
from jax import lax
import jax.experimental.pallas as pl
import jax.experimental.pallas.tpu as pltpu

_cfg = dict(XR=32, R=2, G=7, LK=1, KB1=1, NX=1, G2=7, FS=2, FO=0, PK=1, PW=1, NTRIP=16, PPI=1, XST=1, KXS=0, QMS=0)

S = 2048
D = 640
H = 32
DH = 20
DFF = 1536
NP = H // 2
PR = 2 * DH
PPG = 3
NG = 6
ONE_LANE = 120
TQ = 512
TK = 256
RC = 512
NRC = S // RC
QSCALE = (DH ** -0.5) * math.log2(math.e)
L_MIN = 2.0 ** -40
F32 = jnp.float32
BF16 = jnp.bfloat16
U32 = jnp.uint32
NT = (((1,), (1,)), ((), ()))
NQ = S // TQ
NC = S // TK
CT = TQ // 128
FT = S // NP
XR = _cfg['XR']; R = _cfg['R']; G = _cfg['G']; LK = _cfg['LK']; PPI = _cfg['PPI']
NX = _cfg.get('NX', 0)
XRS = [XR + (16 if ((c + 1) * NX) // NC != (c * NX) // NC else 0) for c in range(NC)]
XOFF = [sum(XRS[:c]) for c in range(NC)]
XK = sum(XRS) + 8 * _cfg.get('KPAD', 0)
OUT_CHUNKS = {0: [(0, 512), (512, 1024), (1024, 1536), (1536, 1920), (1920, 2048)], 1: [(0, 128), (128, 512), (512, 1024), (1024, 1536), (1536, 1920), (1920, 2048)], 2: [(0, 256), (256, 768), (768, 1280), (1280, 1792), (1792, 1920), (1920, 2048)]}[_cfg.get('OC', 0)]


def _kernel(x_hbm, wqkv_hbm, wo_hbm, w1_hbm, w2_hbm, gw_hbm, o_hbm,
            x_v, wqkv_v, wo_v, w1_v, w2_v, gw_v, o_v,
            wkp_scr, wqvt_scr, k_scr, qt_scr, vt_scr, ot_scr, lmin_scr, bb_scr,
            kb0, kb1, qh0, qh1, kst, vst, xst, w1p, w2p, kxf, sems):
    cp_wka = pltpu.make_async_copy(wqkv_hbm.at[:, D:D + 256], wqkv_v.at[:, D:D + 256], sems.at[0])
    cp_wkb = pltpu.make_async_copy(wqkv_hbm.at[:, D + 256:2 * D], wqkv_v.at[:, D + 256:2 * D],
                                   sems.at[11 + len(OUT_CHUNKS)])
    cp_x = [pltpu.make_async_copy(x_hbm.at[0, r * RC:(r + 1) * RC, :], x_v.at[r * RC:(r + 1) * RC, :],
                                  sems.at[1 + r]) for r in range(NRC)]
    cp_wq = pltpu.make_async_copy(wqkv_hbm.at[:, 0:D], wqkv_v.at[:, 0:D], sems.at[5])
    cp_wv = pltpu.make_async_copy(wqkv_hbm.at[:, 2 * D:], wqkv_v.at[:, 2 * D:], sems.at[6])
    cp_w1 = pltpu.make_async_copy(w1_hbm, w1_v, sems.at[7])
    cp_w2 = pltpu.make_async_copy(w2_hbm, w2_v, sems.at[8])
    cp_wo = pltpu.make_async_copy(wo_hbm, wo_v, sems.at[9])
    cp_gw = pltpu.make_async_copy(gw_hbm, gw_v, sems.at[10])
    cp_out = [pltpu.make_async_copy(o_v.at[r0:r1, :], o_hbm.at[0, r0:r1, :], sems.at[11 + i])
              for i, (r0, r1) in enumerate(OUT_CHUNKS)]
    for cp in (cp_wka, cp_x[0], cp_wkb, cp_x[1], cp_x[2], cp_x[3], cp_wv, cp_wq, cp_w1, cp_w2, cp_wo, cp_gw):
        cp.start()

    GW = PPG * PR

    def regroup_wk(groups, c0, c1):
        for rb in range(D // 128):
            wk = wqkv_v[rb * 128:(rb + 1) * 128, D + c0:D + c1].astype(F32)
            for g in groups:
                n = min(GW, D - g * GW)
                piece = jnp.concatenate([wk[:, g * GW - c0:g * GW - c0 + n], jnp.zeros((128, 128 - n), F32)], axis=1)
                wkp_scr[rb * 128:(rb + 1) * 128, g * 128:(g + 1) * 128] = piece.astype(BF16)

    lane = lax.broadcasted_iota(jnp.int32, (RC, 128), 1)
    er = lax.broadcasted_iota(jnp.int32, (16, 128), 0)
    ec = lax.broadcasted_iota(jnp.int32, (16, 128), 1)
    e_k = jnp.where((ec >= er * DH) & (ec < er * DH + DH) & (er < 2 * PPG), 1.0, 0.0).astype(BF16)
    kn_max = [None] * NG

    def k_norm(r, g):
        kf = pltpu.bitcast(k_scr[g, r * RC // 2:(r + 1) * RC // 2, :], BF16).astype(F32)
        kn = lax.dot_general(e_k, (kf * kf).astype(BF16), NT, preferred_element_type=F32)[0:8]
        kn_max[g] = kn if kn_max[g] is None else jnp.maximum(kn_max[g], kn)

    def k_proj(r, g2s=range(NG // 2)):
        xr = x_v[r * RC:(r + 1) * RC, :]
        for g2 in g2s:
            k = jnp.dot(xr, wkp_scr[:, g2 * 256:(g2 + 1) * 256], preferred_element_type=F32)
            for g in (2 * g2, 2 * g2 + 1):
                kg = k[:, (g % 2) * 128:(g % 2 + 1) * 128]
                k_scr[g, r * RC // 2:(r + 1) * RC // 2, :] = pltpu.bitcast(
                    jnp.where(lane == ONE_LANE, 1.0, kg).astype(BF16), U32)
                for c in range(r * RC // TK, (r + 1) * RC // TK):
                    kx = kg[c * TK - r * RC:c * TK - r * RC + XRS[c]].astype(BF16).astype(F32)
                    for pos in range(min(PPG, NP - g * PPG)):
                        kxf[g * PPG + pos, XOFF[c]:XOFF[c] + XRS[c], :] = (
                            pltpu.roll(kx, 128 - pos * PR, axis=1) if pos else kx)
                if r > 0:
                    k_norm(r - 1, g)

    cp_wka.wait()
    cp_x[0].wait()
    regroup_wk((0, 1), 0, 256)
    k_proj(0, (0,))
    cp_wkb.wait()
    regroup_wk((2, 3, 4, 5), 128, D)
    k_proj(0, (1, 2))
    cp_x[1].wait()
    cp_x[2].wait()
    k_proj(1)
    k_proj(2)
    for cp in (cp_x[3], cp_wv, cp_wq):
        cp.wait()
    for cb in range(2 * D // 128):
        src_col = (2 * D if cb < D // 128 else -D) + cb * 128
        wqvt_scr[cb * 128:(cb + 1) * 128, :] = (
            wqkv_v[:, src_col:src_col + 128].astype(F32).T.astype(BF16))
    k_proj(3)

    for r in range(NRC):
        xr = x_v[r * RC:(r + 1) * RC, :]
        cols = slice(r * RC, (r + 1) * RC)
        for half in range(2):
            rows = slice(half * (D // 2), (half + 1) * (D // 2))
            v = lax.dot_general(wqvt_scr[rows, :], xr, NT, preferred_element_type=F32)
            vt_scr[rows, cols] = v.astype(BF16).astype(F32)
            if 2 * r + half < NG:
                k_norm(NRC - 1, 2 * r + half)
    kn_rows = [jnp.max(kn_max[g], axis=1, keepdims=True) for g in range(NG)]
    er = lax.broadcasted_iota(jnp.int32, (H, D), 0)
    ec = lax.broadcasted_iota(jnp.int32, (H, D), 1)
    e_q = jnp.where((ec >= er * DH) & (ec < er * DH + DH), 1.0, 0.0).astype(BF16)
    kn_col = jnp.concatenate([kn_rows[g][0:min(2 * PPG, H - 2 * PPG * g)] for g in range(NG)], axis=0)
    opaque0 = jnp.clip(-(jnp.minimum(jnp.min(kn_col), 0.0).astype(jnp.int32)), 0, DH * XK // 8)
    fence_row = pl.multiple_of((DH * XK // 8 - opaque0) * 8, 8)

    def seal(n):
        return pl.multiple_of((n - jnp.minimum(opaque0, n)) * 8, 8)

    for cp in (cp_w1, cp_w2, cp_wo, cp_gw):
        cp.wait()
    gw = gw_v[...].astype(F32).reshape(1, D)
    for rb in range(D // 128):
        w1p[rb * 64:(rb + 1) * 64, :] = pltpu.bitcast(w1_v[rb * 128:(rb + 1) * 128, :], U32)
    for rb in range(DFF // 128):
        w2p[rb * 64:(rb + 1) * 64, :] = pltpu.bitcast(w2_v[rb * 128:(rb + 1) * 128, :], U32)

    for r in range(NRC):
        xr = x_v[r * RC:(r + 1) * RC, :]
        cols = slice(r * RC, (r + 1) * RC)
        q = lax.dot_general(wqvt_scr[D:, :], xr, NT, preferred_element_type=F32)
        q = (q * QSCALE).astype(BF16).astype(F32)
        qn = jnp.dot(e_q, (q * q).astype(BF16), preferred_element_type=F32)
        nb = -(jnp.sqrt(qn * kn_col) * 1.02)
        nb = nb.astype(BF16).astype(F32)
        for p in range(NP):
            qt_scr[p, 0:PR, cols] = q[p * PR:(p + 1) * PR]
            nbt = nb[8 * (p // 4):8 * (p // 4) + 8]
            if p % 4:
                nbt = pltpu.roll(nbt, 8 - 2 * (p % 4), axis=0)
            qt_scr[p, PR:PR + 8, cols] = nbt
    lmin_scr[...] = jnp.full(lmin_scr.shape, jnp.inf, F32)

    sub_q = lax.broadcasted_iota(jnp.int32, (8, TQ), 0)
    kbs = (kb0, kb1)
    qhs = (qh0, qh1)

    def make_qm(q, nb, pos, hb):
        z8 = jnp.zeros((8, TQ), F32)
        if hb == 0:
            piece = [q[0:16], jnp.where(sub_q < 4, q[16:24], 0.0), z8, z8]
        else:
            piece = [z8, z8, jnp.where(sub_q >= 4, q[0:8], 0.0), q[8:24]]
        rows = []
        for pp in range(PPG):
            rows += [jnp.where(pos == pp, a, jnp.zeros_like(a)) for a in piece]
        rows.append(z8 if nb is None else jnp.where(sub_q == 0, nb, 0.0))
        return jnp.concatenate(rows, axis=0).astype(BF16)

    def v_lhs(r0, hb):
        sub = lax.broadcasted_iota(jnp.int32, (8, S), 0)
        v = vt_scr[pl.ds(r0 + 16 * hb, 24), :]
        if hb == 0:
            return jnp.concatenate([v[0:16], jnp.where(sub == 4, 1.0, v[16:24])], axis=0)
        return jnp.concatenate([jnp.where(sub == 3, 1.0, v[0:8]), v[8:24]], axis=0)

    def write_o(p, hb, cols, acc):
        ot_scr[p, 24 * hb:24 * hb + 24, cols] = acc
        lrow = 20 if hb == 0 else 3
        return acc[lrow:lrow + 1, :]

    def pair_setup(p):
        g = p // PPG
        return g, p - g * PPG, (pl.multiple_of(p * PR, 8) if not isinstance(p, int) else p * PR)

    def build_kb(p, hb, c, d0, d1):
        kx = kxf[p, XOFF[c]:XOFF[c] + XRS[c], :]
        for d in range(d0, d1):
            col = hb * DH + d
            kbs[hb][d * XK + XOFF[c]:d * XK + XOFF[c] + XRS[c], :] = (
                jnp.broadcast_to(kx[:, col:col + 1], (XRS[c], 128)))

    def build_qh(p, hb, qi):
        cols = slice(qi * TQ, (qi + 1) * TQ)
        if _cfg.get('QBB', 0):
            for d in range(DH + 1):
                r = hb * DH + d if d < DH else PR + hb
                qhs[hb][8 * d:8 * d + 8, cols] = jnp.broadcast_to(qt_scr[p, r:r + 1, cols], (8, TQ))
            return
        qhs[hb][0:24, cols] = qt_scr[p, 16 * hb:16 * hb + 24, cols]
        qhs[hb][24:32, cols] = qt_scr[p, PR:PR + 8, cols]

    for c in range(NC):
        build_kb(0, 0, c, 0, DH)
    for qi in range(NQ):
        build_qh(0, 0, qi)

    def stage_x(p):
        rows = pl.ds(pl.multiple_of(p * FT, FT), FT) if not isinstance(p, int) else slice(p * FT, (p + 1) * FT)
        xst[0:FT // 2, :] = pltpu.bitcast(x_v[rows, :], U32)

    stage_x(0)

    def ffn_pieces(rows, pn):
        xsrc = lambda: pltpu.bitcast(xst[0:FT // 2, :], BF16)
        hs = []
        for n in range(DFF // 256):
            hs.append(jnp.maximum(jnp.dot(xsrc(), pltpu.bitcast(w1p[:, n * 256:(n + 1) * 256], BF16), preferred_element_type=F32),
                                  0.0).astype(BF16))
            yield
        hh = jnp.concatenate(hs, axis=1)
        stage_x(pn)
        for n in range(D // 128):
            b = jnp.dot(hh, pltpu.bitcast(w2p[:, n * 128:(n + 1) * 128], BF16), preferred_element_type=F32)
            bb_scr[rows, n * 128:(n + 1) * 128] = b
            yield

    def fast_pairs(it, carry):
        hist = []

        def fence(hb):
            if not hist:
                return
            vals = [a[8 * i:8 * i + 8] for a in hist[-1] for i in range(a.shape[0] // 8)]
            while len(vals) > 1:
                vals = [jnp.maximum(vals[2 * k], vals[2 * k + 1]) for k in range(len(vals) // 2)]
            kbs[hb][pl.ds(fence_row, 8), :] = vals[0]

        def vpu_block(hb, qi, row0, R, G):
            CB = _cfg.get('CB', CT)
            outs = []
            for c0 in range(0, CT, CB):
                accs = []
                for d in range(DH):
                    if d % G == 0:
                        fence(hb)
                    if d == 0:
                        for c in range(CB):
                            col = qi * TQ + (c0 + c) * 128
                            accs.append(jnp.broadcast_to(qhs[hb][24 + hb:25 + hb, col:col + 128], (8 * R, 128)))
                    kb = kbs[hb][d * XK + row0:d * XK + row0 + 8 * R, :]
                    for c in range(CB):
                        col = qi * TQ + (c0 + c) * 128
                        qb = jnp.broadcast_to(qhs[hb][4 * hb + d:4 * hb + d + 1, col:col + 128], (8 * R, 128))
                        accs[c] = accs[c] + kb * qb
                    if d % G == G - 1 - LK or (d == DH - 1 - LK and DH % G):
                        hist.append(list(accs))
                outs += accs
            return jnp.concatenate(outs, axis=1)

        steps = [(j, hb, qi, c) for j in range(PPI) for hb in range(2) for qi in range(NQ) for c in range(NC)]
        ps, accs, qms = {}, {}, {}
        ffn = iter(())
        for t in range(len(steps) + 1):
            if t < len(steps):
                j, hb, qi, c = steps[t]
                p = it * PPI + j if not _cfg.get('STATICP', 0) else 4
                g, pos, r0 = pair_setup(p)
                pn = jnp.minimum(p + 1, NP - 1) if not _cfg.get('STATICP', 0) else 5
                cols = slice(qi * TQ, (qi + 1) * TQ)
                if (hb, qi, c) == (0, 0, 0):
                    kst[0:S // 2, :] = k_scr[g]
                    kst[pl.ds(seal(S // 16), 8), :] = jnp.zeros((8, 128), U32)
                    for hh in range(2):
                        vst[24 * hh:24 * hh + 24, :] = v_lhs(r0, hh)
                    vst[pl.ds(seal(6), 8), :] = jnp.zeros((8, S), F32)
                    for _ in ffn:
                        pass
                    ffn = ffn_pieces(pl.ds(pl.multiple_of(p * FT, FT), FT) if not isinstance(p, int) else slice(p * FT, (p + 1) * FT), pn)
                if t == 0:
                    for _ in range(_cfg.get('FL', 1)):
                        next(ffn, None)
                if c == 0:
                    qms[(j, hb, qi)] = make_qm(qhs[hb][0:24, cols], qhs[hb][24 + hb:25 + hb, cols], pos, hb) if _cfg['QMS'] else make_qm(qt_scr[p, 16 * hb:16 * hb + 24, cols], qt_scr[p, PR + hb:PR + hb + 1, cols], pos, hb)
                s = jnp.dot(pltpu.bitcast(kst[(c * TK + XRS[c]) // 2:(c + 1) * TK // 2, :], BF16), qms[(j, hb, qi)], preferred_element_type=F32)
                sv = [vpu_block(hb, qi, XOFF[c] + b * 8 * R, R, G) for b in range(XR // (8 * R))]
                if XRS[c] > XR:
                    sv.append(vpu_block(hb, qi, XOFF[c] + XR, 2, _cfg.get('G2', 10)))
                if not _cfg.get('KB1', 0):
                    build_kb(p if hb == 0 else pn, 1 - hb, c, qi * DH // NQ, (qi + 1) * DH // NQ)
                elif (qi * NC + c) % NQ == 0:
                    build_kb(p if hb == 0 else pn, 1 - hb, (qi * NC + c) // NQ, 0, DH)
                if c == 0:
                    build_qh(p if hb == 0 else pn, 1 - hb, qi)
                ps[t] = jnp.exp2(jnp.concatenate(sv + [s], axis=0))
                if _cfg.get('PB', 0):
                    ps[t] = ps[t].astype(BF16)
            if t >= 1:
                j, hb, qi, c = steps[t - 1]
                _, _, r0 = pair_setup(it * PPI + j if not _cfg.get('STATICP', 0) else 4)
                d = lax.dot_general(vst[24 * hb:24 * hb + 24, c * TK:(c + 1) * TK], ps.pop(t - 1), (((1,), (0,)), ((), ())), preferred_element_type=F32)
                key = (j, hb, qi)
                accs[key] = d if key not in accs else accs[key] + d
                if c == NC - 1:
                    cols = slice(qi * TQ, (qi + 1) * TQ)
                    l = write_o(it * PPI + j, hb, cols, accs.pop(key))
                    lmin_scr[:, cols] = jnp.minimum(lmin_scr[:, cols], l)
            if (t < 11 - _cfg['FE'] if _cfg.get('FE', 0) else t % _cfg['FS'] == _cfg['FO']):
                next(ffn, None)
        for _ in ffn:
            pass
        return carry

    lax.fori_loop(0, _cfg['NTRIP'] // PPI, fast_pairs, 0)

    safe = jnp.min(lmin_scr[...]) >= L_MIN

    @pl.when(jnp.logical_not(safe))
    def _():
        def slow_tile(it, carry):
            p = it // NQ
            qi = it - p * NQ
            g, pos, r0 = pair_setup(p)
            cols = pl.ds(pl.multiple_of(qi * TQ, TQ), TQ)
            for hb in range(2):
                qm = make_qm(qt_scr[p, 16 * hb:16 * hb + 24, cols], None, pos, hb)
                s = jnp.dot(pltpu.bitcast(k_scr[g], BF16), qm, preferred_element_type=F32)
                m = jnp.max(s, axis=0, keepdims=True)
                pr = jnp.exp2(s - m)
                acc = jnp.dot(v_lhs(r0, hb), pr, preferred_element_type=F32)
                write_o(p, hb, cols, acc)
            return carry
        lax.fori_loop(0, NP * NQ, slow_tile, 0)

    def recip(l):
        r = pl.reciprocal(l, approx=True)
        return r * (2.0 - l * r)

    for i, (r0, r1) in enumerate(OUT_CHUNKS):
        rows = slice(r0, r1)
        sub = lax.broadcasted_iota(jnp.int32, (8, r1 - r0), 0)
        slabs = []
        for p in range(NP):
            oa = ot_scr[p, 0:24, rows]
            ob = ot_scr[p, 24:48, rows]
            oa = oa * recip(oa[20:21, :])
            ob = ob * recip(ob[3:4, :])
            slabs += [oa[0:16], jnp.where(sub < 4, oa[16:24], ob[0:8]), ob[8:24]]
        o = jnp.concatenate(slabs, axis=0).T.astype(BF16)
        a = jnp.dot(o, wo_v[...], preferred_element_type=F32)
        z = jnp.sum(x_v[rows, :].astype(F32) * gw, axis=1, keepdims=True)
        gt = 1.0 / (1.0 + jnp.exp(-z))
        o_v[rows, :] = (gt * a + (1.0 - gt) * bb_scr[rows, :]).astype(o_v.dtype)
        cp_out[i].start()
    for cp in cp_out:
        cp.wait()


@jax.jit
def pallas_gated_mix__softmax_full_mha__dense_activation_relu__prompt_kernel(
        A_x, A_wqkv, A_wo, B_x, B_w1, B_w2, gate_w):
    gw = gate_w
    return pl.pallas_call(
        _kernel,
        in_specs=[pl.BlockSpec(memory_space=pl.ANY)] * 6,
        out_specs=pl.BlockSpec(memory_space=pl.ANY),
        out_shape=jax.ShapeDtypeStruct((1, S, D), A_x.dtype),
        scratch_shapes=[
            pltpu.VMEM((S, D), BF16),
            pltpu.VMEM((D, 3 * D), BF16),
            pltpu.VMEM((D, D), BF16),
            pltpu.VMEM((D, DFF), BF16),
            pltpu.VMEM((DFF, D), BF16),
            pltpu.VMEM((D,), BF16),
            pltpu.VMEM((S, D), BF16),
            pltpu.VMEM((D, NG * 128), BF16),
            pltpu.VMEM((2 * D, D), BF16),
            pltpu.VMEM((NG, S // 2, 128), U32),
            pltpu.VMEM((NP, PR + 8, S), F32),
            pltpu.VMEM((D, S), F32),
            pltpu.VMEM((NP, 48, S), F32),
            pltpu.VMEM((1, S), F32),
            pltpu.VMEM((S, D), F32),
            pltpu.VMEM((DH * XK + 8, 128), F32),
            pltpu.VMEM((DH * XK + 8, 128), F32),
            pltpu.VMEM((168 if _cfg.get('QBB', 0) else 32, S), F32),
            pltpu.VMEM((168 if _cfg.get('QBB', 0) else 32, S), F32),
            pltpu.VMEM((S // 2 + 8, 128), U32),
            pltpu.VMEM((56, S), F32),
            pltpu.VMEM((FT // 2 + 8, D), U32),
            pltpu.VMEM((D // 2, DFF), U32),
            pltpu.VMEM((DFF // 2, D), U32),
            pltpu.VMEM((NP, XK, 128), F32),
            pltpu.SemaphoreType.DMA((12 + len(OUT_CHUNKS),)),
        ],
        compiler_params=pltpu.CompilerParams(vmem_limit_bytes=100 * 1024 * 1024),
    )(A_x, A_wqkv, A_wo, B_w1, B_w2, gw)
```

```python
import math
import jax
import jax.numpy as jnp
from jax import lax
import jax.experimental.pallas as pl
import jax.experimental.pallas.tpu as pltpu

_cfg = dict(G=8, LK=1, FS=4, FL=1, NX=1, NTRIP=16)

S = 2048
D = 640
H = 32
DH = 20
DFF = 1536
NP = H // 2
PR = 2 * DH
PPG = 3
NG = 6
ONE_LANE = 120
TQ = 512
TK = 256
RC = 512
NRC = S // RC
NQ = S // TQ
NC = S // TK
CT = TQ // 128
FT = S // NP
QSCALE = (DH ** -0.5) * math.log2(math.e)
L_MIN = 2.0 ** -40
F32 = jnp.float32
BF16 = jnp.bfloat16
U32 = jnp.uint32
NT = (((1,), (1,)), ((), ()))

VB = 16
G = _cfg['G']
LK = _cfg['LK']
NX = _cfg['NX']
XRS = [32 + (16 if ((c + 1) * NX) // NC != (c * NX) // NC else 0) for c in range(NC)]
XOFF = [sum(XRS[:c]) for c in range(NC)]
XK = sum(XRS)
OUT_CHUNKS = [(0, 512), (512, 1024), (1024, 1536), (1536, 1920), (1920, 2048)]
NSEM = 12 + len(OUT_CHUNKS)


def _kernel(x_hbm, wqkv_hbm, wo_hbm, w1_hbm, w2_hbm, gw_hbm, o_hbm,
            x_v, wqkv_v, wo_v, w1_v, w2_v, gw_v, o_v,
            wkp_scr, wqvt_scr, k_scr, kx_scr, qt_scr, vt_scr, ot_scr, lmin_scr, b_scr,
            kb0, kb1, qh0, qh1, kst, vst, xst, w1p, w2p, accb, sems):
    cp_wka = pltpu.make_async_copy(wqkv_hbm.at[:, D:D + 256], wqkv_v.at[:, D:D + 256], sems.at[0])
    cp_x = [pltpu.make_async_copy(x_hbm.at[0, r * RC:(r + 1) * RC, :], x_v.at[r * RC:(r + 1) * RC, :],
                                  sems.at[1 + r]) for r in range(NRC)]
    cp_wq = pltpu.make_async_copy(wqkv_hbm.at[:, 0:D], wqkv_v.at[:, 0:D], sems.at[5])
    cp_wv = pltpu.make_async_copy(wqkv_hbm.at[:, 2 * D:], wqkv_v.at[:, 2 * D:], sems.at[6])
    cp_w1 = pltpu.make_async_copy(w1_hbm, w1_v, sems.at[7])
    cp_w2 = pltpu.make_async_copy(w2_hbm, w2_v, sems.at[8])
    cp_wo = pltpu.make_async_copy(wo_hbm, wo_v, sems.at[9])
    cp_gw = pltpu.make_async_copy(gw_hbm, gw_v, sems.at[10])
    cp_wkb = pltpu.make_async_copy(wqkv_hbm.at[:, D + 256:2 * D], wqkv_v.at[:, D + 256:2 * D], sems.at[11])
    cp_out = [pltpu.make_async_copy(o_v.at[r0:r1, :], o_hbm.at[0, r0:r1, :], sems.at[12 + i])
              for i, (r0, r1) in enumerate(OUT_CHUNKS)]
    for cp in (cp_wka, cp_x[0], cp_wkb, cp_x[1], cp_x[2], cp_x[3], cp_wv, cp_wq, cp_w1, cp_w2, cp_wo, cp_gw):
        cp.start()

    GW = PPG * PR

    def regroup_wk(groups, c0, c1):
        for rb in range(D // 128):
            wk = pltpu.bitcast(wqkv_v[rb * 128:(rb + 1) * 128, D + c0:D + c1], U32)
            for g in groups:
                n = min(GW, D - g * GW)
                wkp_scr[rb * 64:(rb + 1) * 64, g * 128:(g + 1) * 128] = jnp.concatenate(
                    [wk[:, g * GW - c0:g * GW - c0 + n], jnp.zeros((64, 128 - n), U32)], axis=1)

    lane = lax.broadcasted_iota(jnp.int32, (RC, 128), 1)
    er = lax.broadcasted_iota(jnp.int32, (16, 128), 0)
    ec = lax.broadcasted_iota(jnp.int32, (16, 128), 1)
    e_k = jnp.where((ec >= er * DH) & (ec < er * DH + DH) & (er < 2 * PPG), 1.0, 0.0).astype(BF16)
    kn_max = [None] * NG

    def k_norm(r, g):
        kf = pltpu.bitcast(k_scr[g, r * RC // 2:(r + 1) * RC // 2, :], BF16).astype(F32)
        kn = lax.dot_general(e_k, (kf * kf).astype(BF16), NT, preferred_element_type=F32)[0:8]
        kn_max[g] = kn if kn_max[g] is None else jnp.maximum(kn_max[g], kn)

    def k_proj(r, g2s=range(NG // 2)):
        xr = x_v[r * RC:(r + 1) * RC, :]
        for g2 in g2s:
            w = pltpu.bitcast(wkp_scr[:, g2 * 256:(g2 + 1) * 256], BF16)
            if len(g2s) == 1:
                k = jnp.concatenate([jnp.dot(xr[i * RC // 2:(i + 1) * RC // 2], w, preferred_element_type=F32)
                                     for i in range(2)], axis=0)
            else:
                k = jnp.dot(xr, w, preferred_element_type=F32)
            for g in (2 * g2, 2 * g2 + 1):
                kg = k[:, (g % 2) * 128:(g % 2 + 1) * 128]
                k_scr[g, r * RC // 2:(r + 1) * RC // 2, :] = pltpu.bitcast(
                    jnp.where(lane == ONE_LANE, 1.0, kg).astype(BF16), U32)
                for c in range(r * RC // TK, (r + 1) * RC // TK):
                    kx = kg[c * TK - r * RC:c * TK - r * RC + XRS[c]].astype(BF16).astype(F32)
                    for pos in range(min(PPG, NP - g * PPG)):
                        kx_scr[g * PPG + pos, XOFF[c]:XOFF[c] + XRS[c], :] = (
                            pltpu.roll(kx, 128 - pos * PR, axis=1) if pos else kx)
                if r > 0:
                    k_norm(r - 1, g)

    cp_wka.wait()
    cp_x[0].wait()
    regroup_wk((0, 1), 0, 256)
    k_proj(0, (0,))
    cp_wkb.wait()
    regroup_wk((2, 3, 4, 5), 128, D)
    k_proj(0, (1, 2))
    cp_x[1].wait()
    cp_x[2].wait()
    k_proj(1)
    k_proj(2)
    for cp in (cp_x[3], cp_wv, cp_wq):
        cp.wait()
    for cb in range(2 * D // 128):
        src_col = (2 * D if cb < D // 128 else -D) + cb * 128
        wqvt_scr[cb * 128:(cb + 1) * 128, :] = (
            wqkv_v[:, src_col:src_col + 128].astype(F32).T.astype(BF16))
    k_proj(3)

    for r in range(NRC):
        xr = x_v[r * RC:(r + 1) * RC, :]
        cols = slice(r * RC, (r + 1) * RC)
        for half in range(2):
            rows = slice(half * (D // 2), (half + 1) * (D // 2))
            v = lax.dot_general(wqvt_scr[rows, :], xr, NT, preferred_element_type=F32)
            vt_scr[rows, cols] = v.astype(BF16).astype(F32)
            if 2 * r + half < NG:
                k_norm(NRC - 1, 2 * r + half)
    kn_rows = [jnp.max(kn_max[g], axis=1, keepdims=True) for g in range(NG)]
    kn_col = jnp.concatenate([kn_rows[g][0:min(2 * PPG, H - 2 * PPG * g)] for g in range(NG)], axis=0)
    er = lax.broadcasted_iota(jnp.int32, (H, D), 0)
    ec = lax.broadcasted_iota(jnp.int32, (H, D), 1)
    e_q = jnp.where((ec >= er * DH) & (ec < er * DH + DH), 1.0, 0.0).astype(BF16)

    opaque0 = jnp.clip(-(jnp.minimum(jnp.min(kn_col), 0.0).astype(jnp.int32)), 0, DH * XK // 8)

    def spare(n):
        return pl.ds(pl.multiple_of((n - jnp.minimum(opaque0, n)) * 8, 8), 8)

    for cp in (cp_w1, cp_w2, cp_wo, cp_gw):
        cp.wait()
    for rb in range(D // 128):
        w1p[rb * 64:(rb + 1) * 64, :] = pltpu.bitcast(w1_v[rb * 128:(rb + 1) * 128, :], U32)
    for rb in range(DFF // 128):
        w2p[rb * 64:(rb + 1) * 64, :] = pltpu.bitcast(w2_v[rb * 128:(rb + 1) * 128, :], U32)

    for r in range(NRC):
        xr = x_v[r * RC:(r + 1) * RC, :]
        cols = slice(r * RC, (r + 1) * RC)
        q = lax.dot_general(wqvt_scr[D:, :], xr, NT, preferred_element_type=F32)
        q = (q * QSCALE).astype(BF16).astype(F32)
        qn = jnp.dot(e_q, (q * q).astype(BF16), preferred_element_type=F32)
        nb = -(jnp.sqrt(qn * kn_col) * 1.02)
        nb = nb.astype(BF16).astype(F32)
        for p in range(NP):
            qt_scr[p, 0:PR, cols] = q[p * PR:(p + 1) * PR]
            nbt = nb[8 * (p // 4):8 * (p // 4) + 8]
            if p % 4:
                nbt = pltpu.roll(nbt, 8 - 2 * (p % 4), axis=0)
            qt_scr[p, PR:PR + 8, cols] = nbt
    lmin_scr[...] = jnp.full(lmin_scr.shape, jnp.inf, F32)

    sub_q = lax.broadcasted_iota(jnp.int32, (8, TQ), 0)
    kbs = (kb0, kb1)
    qhs = (qh0, qh1)

    def make_qm(q, nb, pos, hb):
        z8 = jnp.zeros((8, TQ), F32)
        if hb == 0:
            piece = [q[0:16], jnp.where(sub_q < 4, q[16:24], 0.0), z8, z8]
        else:
            piece = [z8, z8, jnp.where(sub_q >= 4, q[0:8], 0.0), q[8:24]]
        rows = []
        for pp in range(PPG):
            rows += [jnp.where(pos == pp, a, jnp.zeros_like(a)) for a in piece]
        rows.append(z8 if nb is None else jnp.where(sub_q == 0, nb, 0.0))
        return jnp.concatenate(rows, axis=0).astype(BF16)

    def v_lhs(r0, hb):
        sub = lax.broadcasted_iota(jnp.int32, (8, S), 0)
        v = vt_scr[pl.ds(r0 + 16 * hb, 24), :]
        if hb == 0:
            return jnp.concatenate([v[0:16], jnp.where(sub == 4, 1.0, v[16:24])], axis=0)
        return jnp.concatenate([jnp.where(sub == 3, 1.0, v[0:8]), v[8:24]], axis=0)

    LROW = (20, 3)

    def pair_setup(p):
        g = p // PPG
        return g, p - g * PPG, pl.multiple_of(p * PR, 8)

    def build_kb(p, hb, c):
        kx = kx_scr[p, XOFF[c]:XOFF[c] + XRS[c], :]
        for d in range(DH):
            col = hb * DH + d
            kbs[hb][d * XK + XOFF[c]:d * XK + XOFF[c] + XRS[c], :] = (
                jnp.broadcast_to(kx[:, col:col + 1], (XRS[c], 128)))

    def build_qh(p, hb, qi):
        cols = slice(qi * TQ, (qi + 1) * TQ)
        qhs[hb][0:24, cols] = qt_scr[p, 16 * hb:16 * hb + 24, cols]
        qhs[hb][24:32, cols] = qt_scr[p, PR:PR + 8, cols]

    def stage_x(rows):
        xst[...] = pltpu.bitcast(x_v[rows, :], U32)

    for c in range(NC):
        build_kb(0, 0, c)
    for qi in range(NQ):
        build_qh(0, 0, qi)
    stage_x(slice(0, FT))

    def ffn_pieces(p, pn):
        rows = pl.ds(pl.multiple_of(p * FT, FT), FT)
        hs = []
        for n in range(DFF // 256):
            h = jnp.dot(pltpu.bitcast(xst[...], BF16), pltpu.bitcast(w1p[:, n * 256:(n + 1) * 256], BF16),
                        preferred_element_type=F32)
            hs.append(jnp.maximum(h, 0.0).astype(BF16))
            yield
        hh = jnp.concatenate(hs, axis=1)
        stage_x(pl.ds(pl.multiple_of(pn * FT, FT), FT))
        for n in range(D // 128):
            b_scr[rows, n * 128:(n + 1) * 128] = jnp.dot(
                hh, pltpu.bitcast(w2p[:, n * 128:(n + 1) * 128], BF16), preferred_element_type=F32)
            yield

    steps = [(hb, qi, c) for hb in range(2) for qi in range(NQ) for c in range(NC)]
    NS = len(steps)

    def fast_pair(p, carry):
        g, pos, r0 = pair_setup(p)
        pn = jnp.minimum(p + 1, NP - 1)
        hist = []

        def fence(hb):
            if not hist:
                return
            vals = [a[8 * i:8 * i + 8] for a in hist[-1] for i in range(VB // 8)]
            while len(vals) > 1:
                vals = [jnp.maximum(vals[2 * k], vals[2 * k + 1]) for k in range(len(vals) // 2)]
            kbs[hb][spare(DH * XK // 8), :] = vals[0]

        def vpu_block(hb, qi, row0):
            accs = []
            for d in range(DH):
                if d % G == 0:
                    fence(hb)
                if d == 0:
                    for c in range(CT):
                        col = qi * TQ + c * 128
                        accs.append(jnp.broadcast_to(qhs[hb][24 + hb:25 + hb, col:col + 128], (VB, 128)))
                kb = kbs[hb][d * XK + row0:d * XK + row0 + VB, :]
                for c in range(CT):
                    col = qi * TQ + c * 128
                    qb = jnp.broadcast_to(qhs[hb][4 * hb + d:4 * hb + d + 1, col:col + 128], (VB, 128))
                    accs[c] = accs[c] + kb * qb
                if d % G == G - 1 - LK or (d == DH - 1 - LK and DH % G):
                    hist.append(list(accs))
            return jnp.concatenate(accs, axis=1)

        kst[0:S // 2, :] = k_scr[g]
        kst[spare(S // 16), :] = jnp.zeros((8, 128), U32)
        for hb in range(2):
            vst[24 * hb:24 * hb + 24, :] = v_lhs(r0, hb)
        vst[spare(6), :] = jnp.zeros((8, S), F32)
        ffn = ffn_pieces(p, pn)
        for _ in range(_cfg['FL']):
            next(ffn, None)
        ps, qms = {}, {}
        for t in range(NS + 1):
            if t < NS:
                hb, qi, c = steps[t]
                cols = slice(qi * TQ, (qi + 1) * TQ)
                if c == 0:
                    qms[(hb, qi)] = make_qm(qt_scr[p, 16 * hb:16 * hb + 24, cols],
                                            qt_scr[p, PR + hb:PR + hb + 1, cols], pos, hb)
                s = jnp.dot(pltpu.bitcast(kst[(c * TK + XRS[c]) // 2:(c + 1) * TK // 2, :], BF16),
                            qms[(hb, qi)], preferred_element_type=F32)
                sv = [vpu_block(hb, qi, XOFF[c] + b * VB) for b in range(XRS[c] // VB)]
                if (qi * NC + c) % NQ == 0:
                    build_kb(p if hb == 0 else pn, 1 - hb, (qi * NC + c) // NQ)
                if c == 0:
                    build_qh(p if hb == 0 else pn, 1 - hb, qi)
                ps[t] = jnp.exp2(jnp.concatenate(sv + [s], axis=0))
            if t >= 1:
                hb, qi, c = steps[t - 1]
                acc = jnp.dot(vst[24 * hb:24 * hb + 24, c * TK:(c + 1) * TK], ps.pop(t - 1),
                              preferred_element_type=F32)
                if c > 0:
                    acc = accb[0:24, :] + acc
                if c < NC - 1:
                    accb[0:24, :] = acc
                    accb[spare(3), :] = jnp.zeros((8, TQ), F32)
                else:
                    cols = slice(qi * TQ, (qi + 1) * TQ)
                    ot_scr[p, 24 * hb:24 * hb + 24, cols] = acc
                    lmin_scr[:, cols] = jnp.minimum(lmin_scr[:, cols], acc[LROW[hb]:LROW[hb] + 1, :])
            if t % _cfg['FS'] == 0:
                next(ffn, None)
        for _ in ffn:
            pass
        return carry

    lax.fori_loop(0, _cfg['NTRIP'], fast_pair, 0)

    safe = jnp.logical_and(jnp.min(lmin_scr[...]) >= L_MIN, opaque0 == 0)

    @pl.when(jnp.logical_not(safe))
    def _():
        def slow_tile(it, carry):
            p = it // NQ
            qi = it - p * NQ
            g, pos, r0 = pair_setup(p)
            cols = pl.ds(pl.multiple_of(qi * TQ, TQ), TQ)
            for hb in range(2):
                qm = make_qm(qt_scr[p, 16 * hb:16 * hb + 24, cols], None, pos, hb)
                s = jnp.dot(pltpu.bitcast(k_scr[g], BF16), qm, preferred_element_type=F32)
                m = jnp.max(s, axis=0, keepdims=True)
                ot_scr[p, 24 * hb:24 * hb + 24, cols] = jnp.dot(
                    v_lhs(r0, hb), jnp.exp2(s - m), preferred_element_type=F32)
            return carry
        lax.fori_loop(0, NP * NQ, slow_tile, 0)

    def recip(l):
        r = pl.reciprocal(l, approx=True)
        return r * (2.0 - l * r)

    gw = gw_v[...].astype(F32).reshape(1, D)
    for i, (r0, r1) in enumerate(OUT_CHUNKS):
        rows = slice(r0, r1)
        sub = lax.broadcasted_iota(jnp.int32, (8, r1 - r0), 0)
        slabs = []
        for p in range(NP):
            oa = ot_scr[p, 0:24, rows]
            ob = ot_scr[p, 24:48, rows]
            oa = oa * recip(oa[LROW[0]:LROW[0] + 1, :])
            ob = ob * recip(ob[LROW[1]:LROW[1] + 1, :])
            slabs += [oa[0:16], jnp.where(sub < 4, oa[16:24], ob[0:8]), ob[8:24]]
        o = jnp.concatenate(slabs, axis=0).T.astype(BF16)
        a = jnp.dot(o, wo_v[...], preferred_element_type=F32)
        z = jnp.sum(x_v[rows, :].astype(F32) * gw, axis=1, keepdims=True)
        gt = 1.0 / (1.0 + jnp.exp(-z))
        o_v[rows, :] = (gt * a + (1.0 - gt) * b_scr[rows, :]).astype(o_v.dtype)
        cp_out[i].start()
    for cp in cp_out:
        cp.wait()


@jax.jit
def pallas_gated_mix__softmax_full_mha__dense_activation_relu__prompt_kernel(
        A_x, A_wqkv, A_wo, B_x, B_w1, B_w2, gate_w):
    return pl.pallas_call(
        _kernel,
        in_specs=[pl.BlockSpec(memory_space=pl.ANY)] * 6,
        out_specs=pl.BlockSpec(memory_space=pl.ANY),
        out_shape=jax.ShapeDtypeStruct((1, S, D), A_x.dtype),
        scratch_shapes=[
            pltpu.VMEM((S, D), BF16),
            pltpu.VMEM((D, 3 * D), BF16),
            pltpu.VMEM((D, D), BF16),
            pltpu.VMEM((D, DFF), BF16),
            pltpu.VMEM((DFF, D), BF16),
            pltpu.VMEM((D,), BF16),
            pltpu.VMEM((S, D), BF16),
            pltpu.VMEM((D // 2, NG * 128), U32),
            pltpu.VMEM((2 * D, D), BF16),
            pltpu.VMEM((NG, S // 2, 128), U32),
            pltpu.VMEM((NP, XK, 128), F32),
            pltpu.VMEM((NP, PR + 8, S), F32),
            pltpu.VMEM((D, S), F32),
            pltpu.VMEM((NP, 48, S), F32),
            pltpu.VMEM((1, S), F32),
            pltpu.VMEM((S, D), F32),
            pltpu.VMEM((DH * XK + 8, 128), F32),
            pltpu.VMEM((DH * XK + 8, 128), F32),
            pltpu.VMEM((32, S), F32),
            pltpu.VMEM((32, S), F32),
            pltpu.VMEM((S // 2 + 8, 128), U32),
            pltpu.VMEM((56, S), F32),
            pltpu.VMEM((FT // 2, D), U32),
            pltpu.VMEM((D // 2, DFF), U32),
            pltpu.VMEM((DFF // 2, D), U32),
            pltpu.VMEM((32, TQ), F32),
            pltpu.SemaphoreType.DMA((NSEM,)),
        ],
        compiler_params=pltpu.CompilerParams(vmem_limit_bytes=100 * 1024 * 1024),
    )(A_x, A_wqkv, A_wo, B_w1, B_w2, gate_w)
```

```python
import math
import jax
import jax.numpy as jnp
from jax import lax
import jax.experimental.pallas as pl
import jax.experimental.pallas.tpu as pltpu

S = 2048
D = 640
H = 32
DH = 20
DFF = 1536
NP = H // 2
PR = 2 * DH
PPG = 3
NG = 6
ONE_LANE = 120
TQ = 512
TK = 256
RC = 512
NRC = S // RC
NQ = S // TQ
NC = S // TK
CT = TQ // 128
FT = S // NP
QSCALE = (DH ** -0.5) * math.log2(math.e)
L_MIN = 2.0 ** -40
F32 = jnp.float32
BF16 = jnp.bfloat16
U32 = jnp.uint32
NT = (((1,), (1,)), ((), ()))

VB = 16
G = 7
LK = 2
FFN_EVERY = 4
XRS = [32] * (NC - 1) + [48]
XOFF = [sum(XRS[:c]) for c in range(NC)]
XK = sum(XRS)


def _stored_order(c):
    return list(range(XRS[c] // 8)) + list(range(TK // 8 - 1, XRS[c] // 8 - 1, -1))


def _to_stored(x, c):
    return [x[8 * j:8 * j + 8] for j in _stored_order(c)]


def _to_keys(x, c):
    o = _stored_order(c)
    return [x[8 * o.index(j):8 * o.index(j) + 8] for j in range(TK // 8)]


OUT_CHUNKS = [(0, 512), (512, 1024), (1024, 1536), (1536, 1920), (1920, 2048)]
NSEM = 12 + len(OUT_CHUNKS)


def _kernel(x_hbm, wqkv_hbm, wo_hbm, w1_hbm, w2_hbm, gw_hbm, o_hbm,
            x_v, wqkv_v, wo_v, w1_v, w2_v, gw_v, o_v,
            wkp_scr, wqvt_scr, k_scr, kx_scr, qt_scr, vt_scr, ot_scr, lmin_scr, b_scr,
            kb0, kb1, qh0, qh1, kst, vst, xst, w1p, w2p, accb, sems):
    cp_wka = pltpu.make_async_copy(wqkv_hbm.at[:, D:D + 256], wqkv_v.at[:, D:D + 256], sems.at[0])
    cp_x = [pltpu.make_async_copy(x_hbm.at[0, r * RC:(r + 1) * RC, :], x_v.at[r * RC:(r + 1) * RC, :],
                                  sems.at[1 + r]) for r in range(NRC)]
    cp_wq = pltpu.make_async_copy(wqkv_hbm.at[:, 0:D], wqkv_v.at[:, 0:D], sems.at[5])
    cp_wv = pltpu.make_async_copy(wqkv_hbm.at[:, 2 * D:], wqkv_v.at[:, 2 * D:], sems.at[6])
    cp_w1 = pltpu.make_async_copy(w1_hbm, w1_v, sems.at[7])
    cp_w2 = pltpu.make_async_copy(w2_hbm, w2_v, sems.at[8])
    cp_wo = pltpu.make_async_copy(wo_hbm, wo_v, sems.at[9])
    cp_gw = pltpu.make_async_copy(gw_hbm, gw_v, sems.at[10])
    cp_wkb = pltpu.make_async_copy(wqkv_hbm.at[:, D + 256:2 * D], wqkv_v.at[:, D + 256:2 * D], sems.at[11])
    cp_out = [pltpu.make_async_copy(o_v.at[r0:r1, :], o_hbm.at[0, r0:r1, :], sems.at[12 + i])
              for i, (r0, r1) in enumerate(OUT_CHUNKS)]
    for cp in (cp_wka, cp_x[0], cp_wkb, cp_x[1], cp_x[2], cp_x[3], cp_wv, cp_wq, cp_w1, cp_w2, cp_wo, cp_gw):
        cp.start()

    GW = PPG * PR

    def regroup_wk(groups, c0, c1):
        for rb in range(D // 128):
            wk = pltpu.bitcast(wqkv_v[rb * 128:(rb + 1) * 128, D + c0:D + c1], U32)
            for g in groups:
                n = min(GW, D - g * GW)
                wkp_scr[rb * 64:(rb + 1) * 64, g * 128:(g + 1) * 128] = jnp.concatenate(
                    [wk[:, g * GW - c0:g * GW - c0 + n], jnp.zeros((64, 128 - n), U32)], axis=1)

    lane = lax.broadcasted_iota(jnp.int32, (RC, 128), 1)
    er = lax.broadcasted_iota(jnp.int32, (16, 128), 0)
    ec = lax.broadcasted_iota(jnp.int32, (16, 128), 1)
    e_k = jnp.where((ec >= er * DH) & (ec < er * DH + DH) & (er < 2 * PPG), 1.0, 0.0).astype(BF16)
    kn_max = [None] * NG

    def k_norm(r, g):
        kf = pltpu.bitcast(k_scr[g, r * RC // 2:(r + 1) * RC // 2, :], BF16).astype(F32)
        kn = lax.dot_general(e_k, (kf * kf).astype(BF16), NT, preferred_element_type=F32)[0:8]
        kn_max[g] = kn if kn_max[g] is None else jnp.maximum(kn_max[g], kn)

    def k_proj(r, g2s=range(NG // 2)):
        xr = x_v[r * RC:(r + 1) * RC, :]
        for g2 in g2s:
            w = pltpu.bitcast(wkp_scr[:, g2 * 256:(g2 + 1) * 256], BF16)
            if len(g2s) == 1:
                k = jnp.concatenate([jnp.dot(xr[i * RC // 2:(i + 1) * RC // 2], w, preferred_element_type=F32)
                                     for i in range(2)], axis=0)
            else:
                k = jnp.dot(xr, w, preferred_element_type=F32)
            for g in (2 * g2, 2 * g2 + 1):
                kg = k[:, (g % 2) * 128:(g % 2 + 1) * 128]
                k1 = jnp.where(lane == ONE_LANE, 1.0, kg)
                k1 = jnp.concatenate(
                    [a for c in range(r * RC // TK, (r + 1) * RC // TK)
                     for a in _to_stored(k1[c * TK - r * RC:(c + 1) * TK - r * RC], c)], axis=0)
                k_scr[g, r * RC // 2:(r + 1) * RC // 2, :] = pltpu.bitcast(k1.astype(BF16), U32)
                for c in range(r * RC // TK, (r + 1) * RC // TK):
                    kx = k1[c * TK - r * RC:c * TK - r * RC + XRS[c]].astype(BF16).astype(F32)
                    for pos in range(min(PPG, NP - g * PPG)):
                        kx_scr[g * PPG + pos, XOFF[c]:XOFF[c] + XRS[c], :] = (
                            pltpu.roll(kx, 128 - pos * PR, axis=1) if pos else kx)
                if r > 0:
                    k_norm(r - 1, g)

    cp_wka.wait()
    cp_x[0].wait()
    regroup_wk((0, 1), 0, 256)
    k_proj(0, (0,))
    cp_wkb.wait()
    regroup_wk((2, 3, 4, 5), 128, D)
    k_proj(0, (1, 2))
    cp_x[1].wait()
    cp_x[2].wait()
    k_proj(1)
    k_proj(2)
    for cp in (cp_x[3], cp_wv, cp_wq):
        cp.wait()
    for cb in range(2 * D // 128):
        src_col = (2 * D if cb < D // 128 else -D) + cb * 128
        wqvt_scr[cb * 128:(cb + 1) * 128, :] = (
            wqkv_v[:, src_col:src_col + 128].astype(F32).T.astype(BF16))
    k_proj(3)

    for r in range(NRC):
        xr = x_v[r * RC:(r + 1) * RC, :]
        cols = slice(r * RC, (r + 1) * RC)
        for half in range(2):
            rows = slice(half * (D // 2), (half + 1) * (D // 2))
            v = lax.dot_general(wqvt_scr[rows, :], xr, NT, preferred_element_type=F32)
            vt_scr[rows, cols] = v.astype(BF16).astype(F32)
            if 2 * r + half < NG:
                k_norm(NRC - 1, 2 * r + half)
    kn_rows = [jnp.max(kn_max[g], axis=1, keepdims=True) for g in range(NG)]
    kn_col = jnp.concatenate([kn_rows[g][0:min(2 * PPG, H - 2 * PPG * g)] for g in range(NG)], axis=0)
    er = lax.broadcasted_iota(jnp.int32, (H, D), 0)
    ec = lax.broadcasted_iota(jnp.int32, (H, D), 1)
    e_q = jnp.where((ec >= er * DH) & (ec < er * DH + DH), 1.0, 0.0).astype(BF16)

    opaque0 = jnp.clip(-(jnp.minimum(jnp.min(kn_col), 0.0).astype(jnp.int32)), 0, DH * XK // 8)

    def spare(n):
        return pl.ds(pl.multiple_of((n - jnp.minimum(opaque0, n)) * 8, 8), 8)

    for cp in (cp_w1, cp_w2, cp_wo, cp_gw):
        cp.wait()
    for rb in range(D // 128):
        w1p[rb * 64:(rb + 1) * 64, :] = pltpu.bitcast(w1_v[rb * 128:(rb + 1) * 128, :], U32)
    for rb in range(DFF // 128):
        w2p[rb * 64:(rb + 1) * 64, :] = pltpu.bitcast(w2_v[rb * 128:(rb + 1) * 128, :], U32)

    for r in range(NRC):
        xr = x_v[r * RC:(r + 1) * RC, :]
        cols = slice(r * RC, (r + 1) * RC)
        q = lax.dot_general(wqvt_scr[D:, :], xr, NT, preferred_element_type=F32)
        q = (q * QSCALE).astype(BF16).astype(F32)
        qn = jnp.dot(e_q, (q * q).astype(BF16), preferred_element_type=F32)
        nb = -(jnp.sqrt(qn * kn_col) * 1.02)
        nb = nb.astype(BF16).astype(F32)
        for p in range(NP):
            qt_scr[p, 0:PR, cols] = q[p * PR:(p + 1) * PR]
            nbt = nb[8 * (p // 4):8 * (p // 4) + 8]
            if p % 4:
                nbt = pltpu.roll(nbt, 8 - 2 * (p % 4), axis=0)
            qt_scr[p, PR:PR + 8, cols] = nbt
    lmin_scr[...] = jnp.full(lmin_scr.shape, jnp.inf, F32)

    sub_q = lax.broadcasted_iota(jnp.int32, (8, TQ), 0)
    kbs = (kb0, kb1)
    qhs = (qh0, qh1)

    def make_qm(q, nb, pos, hb):
        z8 = jnp.zeros((8, TQ), F32)
        if hb == 0:
            piece = [q[0:16], jnp.where(sub_q < 4, q[16:24], 0.0), z8, z8]
        else:
            piece = [z8, z8, jnp.where(sub_q >= 4, q[0:8], 0.0), q[8:24]]
        rows = []
        for pp in range(PPG):
            rows += [jnp.where(pos == pp, a, jnp.zeros_like(a)) for a in piece]
        rows.append(z8 if nb is None else jnp.where(sub_q == 0, nb, 0.0))
        return jnp.concatenate(rows, axis=0).astype(BF16)

    def v_lhs(r0, hb):
        sub = lax.broadcasted_iota(jnp.int32, (8, S), 0)
        v = vt_scr[pl.ds(r0 + 16 * hb, 24), :]
        if hb == 0:
            return jnp.concatenate([v[0:16], jnp.where(sub == 4, 1.0, v[16:24])], axis=0)
        return jnp.concatenate([jnp.where(sub == 3, 1.0, v[0:8]), v[8:24]], axis=0)

    LROW = (20, 3)

    def pair_setup(p):
        g = p // PPG
        return g, p - g * PPG, pl.multiple_of(p * PR, 8)

    def build_kb(p, hb, c):
        kx = kx_scr[p, XOFF[c]:XOFF[c] + XRS[c], :]
        for d in range(DH):
            col = hb * DH + d
            kbs[hb][d * XK + XOFF[c]:d * XK + XOFF[c] + XRS[c], :] = (
                jnp.broadcast_to(kx[:, col:col + 1], (XRS[c], 128)))

    def build_qh(p, hb, qi):
        cols = slice(qi * TQ, (qi + 1) * TQ)
        qhs[hb][0:24, cols] = qt_scr[p, 16 * hb:16 * hb + 24, cols]
        qhs[hb][24:32, cols] = qt_scr[p, PR:PR + 8, cols]

    def stage_x(rows):
        xst[...] = pltpu.bitcast(x_v[rows, :], U32)

    for c in range(NC):
        build_kb(0, 0, c)
    for qi in range(NQ):
        build_qh(0, 0, qi)
    stage_x(slice(0, FT))
    kst[...] = k_scr[0]

    def ffn_pieces(p, pn):
        rows = pl.ds(pl.multiple_of(p * FT, FT), FT)
        hs = []
        for n in range(DFF // 256):
            h = jnp.dot(pltpu.bitcast(xst[...], BF16), pltpu.bitcast(w1p[:, n * 256:(n + 1) * 256], BF16),
                        preferred_element_type=F32)
            hs.append(jnp.maximum(h, 0.0).astype(BF16))
            yield
        hh = jnp.concatenate(hs, axis=1)
        stage_x(pl.ds(pl.multiple_of(pn * FT, FT), FT))
        for n in range(D // 128):
            b_scr[rows, n * 128:(n + 1) * 128] = jnp.dot(
                hh, pltpu.bitcast(w2p[:, n * 128:(n + 1) * 128], BF16), preferred_element_type=F32)
            yield

    steps = [(hb, qi, c) for hb in range(2) for qi in range(NQ) for c in range(NC)]
    NS = len(steps)

    def fast_pair(p, carry):
        g, pos, r0 = pair_setup(p)
        pn = jnp.minimum(p + 1, NP - 1)
        hist = []

        def fence(hb):
            if not hist:
                return
            vals = [a[8 * i:8 * i + 8] for a in hist[-1] for i in range(VB // 8)]
            while len(vals) > 1:
                vals = [jnp.maximum(vals[2 * k], vals[2 * k + 1]) for k in range(len(vals) // 2)]
            kbs[hb][spare(DH * XK // 8), :] = vals[0]

        def vpu_block(hb, qi, row0):
            accs = []
            for d in range(DH):
                if d % G == 0:
                    fence(hb)
                if d == 0:
                    for c in range(CT):
                        col = qi * TQ + c * 128
                        accs.append(jnp.broadcast_to(qhs[hb][24 + hb:25 + hb, col:col + 128], (VB, 128)))
                kb = kbs[hb][d * XK + row0:d * XK + row0 + VB, :]
                for c in range(CT):
                    col = qi * TQ + c * 128
                    qb = jnp.broadcast_to(qhs[hb][4 * hb + d:4 * hb + d + 1, col:col + 128], (VB, 128))
                    accs[c] = accs[c] + kb * qb
                if d % G == G - 1 - LK or d == DH - 1 - LK:
                    hist.append(list(accs))
            return jnp.concatenate(accs, axis=1)

        @pl.when(jnp.logical_and(pos == 0, p > 0))
        def _():
            kst[...] = k_scr[g]

        for hb in range(2):
            vst[24 * hb:24 * hb + 24, :] = v_lhs(r0, hb)
        vst[spare(6), :] = jnp.zeros((8, S), F32)
        ffn = ffn_pieces(p, pn)
        next(ffn)
        ps, qms = {}, {}
        for t in range(NS + 1):
            if t < NS:
                hb, qi, c = steps[t]
                cols = slice(qi * TQ, (qi + 1) * TQ)
                if c == 0:
                    qms[(hb, qi)] = make_qm(qt_scr[p, 16 * hb:16 * hb + 24, cols],
                                            qt_scr[p, PR + hb:PR + hb + 1, cols], pos, hb)
                s = jnp.dot(pltpu.bitcast(kst[(c * TK + XRS[c]) // 2:(c + 1) * TK // 2, :], BF16),
                            qms[(hb, qi)], preferred_element_type=F32)
                sv = [vpu_block(hb, qi, XOFF[c] + b * VB) for b in range(XRS[c] // VB)]
                if (qi * NC + c) % NQ == 0:
                    build_kb(p if hb == 0 else pn, 1 - hb, (qi * NC + c) // NQ)
                if c == 0:
                    build_qh(p if hb == 0 else pn, 1 - hb, qi)
                s = jnp.concatenate(sv + [s], axis=0)
                ps[t] = jnp.exp2(jnp.concatenate(_to_keys(s, c), axis=0))
            if t >= 1:
                hb, qi, c = steps[t - 1]
                acc = jnp.dot(vst[24 * hb:24 * hb + 24, c * TK:(c + 1) * TK], ps.pop(t - 1),
                              preferred_element_type=F32)
                if c > 0:
                    acc = jnp.concatenate([accb[24 * j:24 * j + 24, :] for j in range(CT)], axis=1) + acc
                if c < NC - 1:
                    for j in range(CT):
                        accb[24 * j:24 * j + 24, :] = acc[:, 128 * j:128 * j + 128]
                    accb[spare(3 * CT), :] = jnp.zeros((8, 128), F32)
                else:
                    cols = slice(qi * TQ, (qi + 1) * TQ)
                    ot_scr[p, 24 * hb:24 * hb + 24, cols] = acc
                    lmin_scr[:, cols] = jnp.minimum(lmin_scr[:, cols], acc[LROW[hb]:LROW[hb] + 1, :])
            if t % FFN_EVERY == 0:
                next(ffn, None)
        for _ in ffn:
            pass
        return carry

    lax.fori_loop(0, NP, fast_pair, 0)

    safe = jnp.logical_and(jnp.min(lmin_scr[...]) >= L_MIN, opaque0 == 0)

    @pl.when(jnp.logical_not(safe))
    def _():
        def slow_tile(it, carry):
            p = it // NQ
            qi = it - p * NQ
            g, pos, r0 = pair_setup(p)
            cols = pl.ds(pl.multiple_of(qi * TQ, TQ), TQ)
            for hb in range(2):
                qm = make_qm(qt_scr[p, 16 * hb:16 * hb + 24, cols], None, pos, hb)
                s = jnp.dot(pltpu.bitcast(k_scr[g], BF16), qm, preferred_element_type=F32)
                s = jnp.concatenate([a for c in range(NC) for a in _to_keys(s[c * TK:(c + 1) * TK], c)], axis=0)
                m = jnp.max(s, axis=0, keepdims=True)
                ot_scr[p, 24 * hb:24 * hb + 24, cols] = jnp.dot(
                    v_lhs(r0, hb), jnp.exp2(s - m), preferred_element_type=F32)
            return carry
        lax.fori_loop(0, NP * NQ, slow_tile, 0)

    def recip(l):
        r = pl.reciprocal(l, approx=True)
        return r * (2.0 - l * r)

    gw = gw_v[...].astype(F32).reshape(1, D)
    for i, (r0, r1) in enumerate(OUT_CHUNKS):
        rows = slice(r0, r1)
        sub = lax.broadcasted_iota(jnp.int32, (8, r1 - r0), 0)
        slabs = []
        for p in range(NP):
            oa = ot_scr[p, 0:24, rows]
            ob = ot_scr[p, 24:48, rows]
            oa = oa * recip(oa[LROW[0]:LROW[0] + 1, :])
            ob = ob * recip(ob[LROW[1]:LROW[1] + 1, :])
            slabs += [oa[0:16], jnp.where(sub < 4, oa[16:24], ob[0:8]), ob[8:24]]
        o = jnp.concatenate(slabs, axis=0).T.astype(BF16)
        a = jnp.dot(o, wo_v[...], preferred_element_type=F32)
        z = jnp.sum(x_v[rows, :].astype(F32) * gw, axis=1, keepdims=True)
        gt = 1.0 / (1.0 + jnp.exp(-z))
        o_v[rows, :] = (gt * a + (1.0 - gt) * b_scr[rows, :]).astype(o_v.dtype)
        cp_out[i].start()
    for cp in cp_out:
        cp.wait()


@jax.jit
def pallas_gated_mix__softmax_full_mha__dense_activation_relu__prompt_kernel(
        A_x, A_wqkv, A_wo, B_x, B_w1, B_w2, gate_w):
    return pl.pallas_call(
        _kernel,
        in_specs=[pl.BlockSpec(memory_space=pl.ANY)] * 6,
        out_specs=pl.BlockSpec(memory_space=pl.ANY),
        out_shape=jax.ShapeDtypeStruct((1, S, D), A_x.dtype),
        scratch_shapes=[
            pltpu.VMEM((S, D), BF16),
            pltpu.VMEM((D, 3 * D), BF16),
            pltpu.VMEM((D, D), BF16),
            pltpu.VMEM((D, DFF), BF16),
            pltpu.VMEM((DFF, D), BF16),
            pltpu.VMEM((D,), BF16),
            pltpu.VMEM((S, D), BF16),
            pltpu.VMEM((D // 2, NG * 128), U32),
            pltpu.VMEM((2 * D, D), BF16),
            pltpu.VMEM((NG, S // 2, 128), U32),
            pltpu.VMEM((NP, XK, 128), F32),
            pltpu.VMEM((NP, PR + 8, S), F32),
            pltpu.VMEM((D, S), F32),
            pltpu.VMEM((NP, 48, S), F32),
            pltpu.VMEM((1, S), F32),
            pltpu.VMEM((S, D), F32),
            pltpu.VMEM((DH * XK + 8, 128), F32),
            pltpu.VMEM((DH * XK + 8, 128), F32),
            pltpu.VMEM((32, S), F32),
            pltpu.VMEM((32, S), F32),
            pltpu.VMEM((S // 2, 128), U32),
            pltpu.VMEM((56, S), F32),
            pltpu.VMEM((FT // 2, D), U32),
            pltpu.VMEM((D // 2, DFF), U32),
            pltpu.VMEM((DFF // 2, D), U32),
            pltpu.VMEM((24 * CT + 8, 128), F32),
            pltpu.SemaphoreType.DMA((NSEM,)),
        ],
        compiler_params=pltpu.CompilerParams(vmem_limit_bytes=100 * 1024 * 1024),
    )(A_x, A_wqkv, A_wo, B_w1, B_w2, gate_w)
```

```python
import math
import jax
import jax.numpy as jnp
from jax import lax
import jax.experimental.pallas as pl
import jax.experimental.pallas.tpu as pltpu

S = 2048
D = 640
H = 32
DH = 20
DFF = 1536
NP = H // 2
PR = 2 * DH
PPG = 3
NG = 6
ONE_LANE = 120
TQ = 512
TK = 256
RC = 512
NRC = S // RC
NQ = S // TQ
NC = S // TK
CT = TQ // 128
FT = S // NP
QSCALE = (DH ** -0.5) * math.log2(math.e)
L_MIN = 2.0 ** -40
F32 = jnp.float32
BF16 = jnp.bfloat16
U32 = jnp.uint32
NT = (((1,), (1,)), ((), ()))

VB = 16
G = 7
LK = 2
FFN_EVERY = 4
XRS = [32] * (NC - 1) + [48]
XOFF = [sum(XRS[:c]) for c in range(NC)]
XK = sum(XRS)


def _stored_order(c):
    return list(range(XRS[c] // 8)) + list(range(TK // 8 - 1, XRS[c] // 8 - 1, -1))


def _to_stored(x, c):
    return [x[8 * j:8 * j + 8] for j in _stored_order(c)]


def _to_keys(x, c):
    o = _stored_order(c)
    return [x[8 * o.index(j):8 * o.index(j) + 8] for j in range(TK // 8)]


OUT_CHUNKS = [(0, 512), (512, 1024), (1024, 1536), (1536, 1920), (1920, 2048)]
NSEM = 12 + len(OUT_CHUNKS)


def _kernel(x_hbm, wqkv_hbm, wo_hbm, w1_hbm, w2_hbm, gw_hbm, o_hbm,
            x_v, wqkv_v, wo_v, w1_v, w2_v, gw_v, o_v,
            wkp_scr, wqvt_scr, k_scr, kx_scr, qt_scr, vt_scr, ot_scr, lmin_scr, b_scr,
            kb0, kb1, qh, kst, vst, xst, w1p, w2p, accb, sems):
    cp_wka = pltpu.make_async_copy(wqkv_hbm.at[:, D:D + 256], wqkv_v.at[:, D:D + 256], sems.at[0])
    cp_x = [pltpu.make_async_copy(x_hbm.at[0, r * RC:(r + 1) * RC, :], x_v.at[r * RC:(r + 1) * RC, :],
                                  sems.at[1 + r]) for r in range(NRC)]
    cp_wq = pltpu.make_async_copy(wqkv_hbm.at[:, 0:D], wqkv_v.at[:, 0:D], sems.at[5])
    cp_wv = pltpu.make_async_copy(wqkv_hbm.at[:, 2 * D:], wqkv_v.at[:, 2 * D:], sems.at[6])
    cp_w1 = pltpu.make_async_copy(w1_hbm, w1_v, sems.at[7])
    cp_w2 = pltpu.make_async_copy(w2_hbm, w2_v, sems.at[8])
    cp_wo = pltpu.make_async_copy(wo_hbm, wo_v, sems.at[9])
    cp_gw = pltpu.make_async_copy(gw_hbm, gw_v, sems.at[10])
    cp_wkb = pltpu.make_async_copy(wqkv_hbm.at[:, D + 256:2 * D], wqkv_v.at[:, D + 256:2 * D], sems.at[11])
    cp_out = [pltpu.make_async_copy(o_v.at[r0:r1, :], o_hbm.at[0, r0:r1, :], sems.at[12 + i])
              for i, (r0, r1) in enumerate(OUT_CHUNKS)]
    for cp in (cp_wka, cp_x[0], cp_wkb, cp_x[1], cp_x[2], cp_x[3], cp_wv, cp_wq, cp_w1, cp_w2, cp_wo, cp_gw):
        cp.start()

    GW = PPG * PR

    def regroup_wk(groups, c0, c1):
        for rb in range(D // 128):
            wk = pltpu.bitcast(wqkv_v[rb * 128:(rb + 1) * 128, D + c0:D + c1], U32)
            for g in groups:
                n = min(GW, D - g * GW)
                wkp_scr[rb * 64:(rb + 1) * 64, g * 128:(g + 1) * 128] = jnp.concatenate(
                    [wk[:, g * GW - c0:g * GW - c0 + n], jnp.zeros((64, 128 - n), U32)], axis=1)

    lane = lax.broadcasted_iota(jnp.int32, (RC, 128), 1)
    er = lax.broadcasted_iota(jnp.int32, (16, 128), 0)
    ec = lax.broadcasted_iota(jnp.int32, (16, 128), 1)
    e_k = jnp.where((ec >= er * DH) & (ec < er * DH + DH) & (er < 2 * PPG), 1.0, 0.0).astype(BF16)
    kn_max = [None] * NG

    def k_norm(r, g):
        kf = pltpu.bitcast(k_scr[g, r * RC // 2:(r + 1) * RC // 2, :], BF16).astype(F32)
        kn = lax.dot_general(e_k, (kf * kf).astype(BF16), NT, preferred_element_type=F32)[0:8]
        kn_max[g] = kn if kn_max[g] is None else jnp.maximum(kn_max[g], kn)

    def k_proj(r, g2s=range(NG // 2)):
        xr = x_v[r * RC:(r + 1) * RC, :]
        for g2 in g2s:
            w = pltpu.bitcast(wkp_scr[:, g2 * 256:(g2 + 1) * 256], BF16)
            if len(g2s) == 1:
                k = jnp.concatenate([jnp.dot(xr[i * RC // 2:(i + 1) * RC // 2], w, preferred_element_type=F32)
                                     for i in range(2)], axis=0)
            else:
                k = jnp.dot(xr, w, preferred_element_type=F32)
            for g in (2 * g2, 2 * g2 + 1):
                kg = k[:, (g % 2) * 128:(g % 2 + 1) * 128]
                k1 = jnp.where(lane == ONE_LANE, 1.0, kg)
                k1 = jnp.concatenate(
                    [a for c in range(r * RC // TK, (r + 1) * RC // TK)
                     for a in _to_stored(k1[c * TK - r * RC:(c + 1) * TK - r * RC], c)], axis=0)
                k_scr[g, r * RC // 2:(r + 1) * RC // 2, :] = pltpu.bitcast(k1.astype(BF16), U32)
                for c in range(r * RC // TK, (r + 1) * RC // TK):
                    kx = k1[c * TK - r * RC:c * TK - r * RC + XRS[c]].astype(BF16).astype(F32)
                    for pos in range(min(PPG, NP - g * PPG)):
                        kx_scr[g * PPG + pos, XOFF[c]:XOFF[c] + XRS[c], :] = (
                            pltpu.roll(kx, 128 - pos * PR, axis=1) if pos else kx)
                if r > 0:
                    k_norm(r - 1, g)

    cp_wka.wait()
    cp_x[0].wait()
    regroup_wk((0, 1), 0, 256)
    k_proj(0, (0,))
    cp_wkb.wait()
    regroup_wk((2, 3, 4, 5), 128, D)
    k_proj(0, (1, 2))
    cp_x[1].wait()
    cp_x[2].wait()
    k_proj(1)
    k_proj(2)
    for cp in (cp_x[3], cp_wv, cp_wq):
        cp.wait()
    for cb in range(2 * D // 128):
        src_col = (2 * D if cb < D // 128 else -D) + cb * 128
        wqvt_scr[cb * 128:(cb + 1) * 128, :] = (
            wqkv_v[:, src_col:src_col + 128].astype(F32).T.astype(BF16))
    k_proj(3)

    for r in range(NRC):
        xr = x_v[r * RC:(r + 1) * RC, :]
        cols = slice(r * RC, (r + 1) * RC)
        for half in range(2):
            rows = slice(half * (D // 2), (half + 1) * (D // 2))
            v = lax.dot_general(wqvt_scr[rows, :], xr, NT, preferred_element_type=F32)
            vt_scr[rows, cols] = v.astype(BF16).astype(F32)
            if 2 * r + half < NG:
                k_norm(NRC - 1, 2 * r + half)
    kn_rows = [jnp.max(kn_max[g], axis=1, keepdims=True) for g in range(NG)]
    kn_col = jnp.concatenate([kn_rows[g][0:min(2 * PPG, H - 2 * PPG * g)] for g in range(NG)], axis=0)
    er = lax.broadcasted_iota(jnp.int32, (H, D), 0)
    ec = lax.broadcasted_iota(jnp.int32, (H, D), 1)
    e_q = jnp.where((ec >= er * DH) & (ec < er * DH + DH), 1.0, 0.0).astype(BF16)

    opaque0 = jnp.clip(-(jnp.minimum(jnp.min(kn_col), 0.0).astype(jnp.int32)), 0, DH * XK // 8)

    def spare(n):
        return pl.ds(pl.multiple_of((n - jnp.minimum(opaque0, n)) * 8, 8), 8)

    kb_spare, v_spare, acc_spare = spare(DH * XK // 8), spare(6), spare(3 * CT)

    for cp in (cp_w1, cp_w2, cp_wo, cp_gw):
        cp.wait()
    for rb in range(D // 128):
        w1p[rb * 64:(rb + 1) * 64, :] = pltpu.bitcast(w1_v[rb * 128:(rb + 1) * 128, :], U32)
    for rb in range(DFF // 128):
        w2p[rb * 64:(rb + 1) * 64, :] = pltpu.bitcast(w2_v[rb * 128:(rb + 1) * 128, :], U32)

    for r in range(NRC):
        xr = x_v[r * RC:(r + 1) * RC, :]
        cols = slice(r * RC, (r + 1) * RC)
        q = lax.dot_general(wqvt_scr[D:, :], xr, NT, preferred_element_type=F32)
        q = (q * QSCALE).astype(BF16).astype(F32)
        qn = jnp.dot(e_q, (q * q).astype(BF16), preferred_element_type=F32)
        nb = -(jnp.sqrt(qn * kn_col) * 1.02)
        nb = nb.astype(BF16).astype(F32)
        for p in range(NP):
            qt_scr[p, 0:PR, cols] = q[p * PR:(p + 1) * PR]
            nbt = nb[8 * (p // 4):8 * (p // 4) + 8]
            if p % 4:
                nbt = pltpu.roll(nbt, 8 - 2 * (p % 4), axis=0)
            qt_scr[p, PR:PR + 8, cols] = nbt
    lmin_scr[...] = jnp.full(lmin_scr.shape, jnp.inf, F32)

    sub_q = lax.broadcasted_iota(jnp.int32, (8, TQ), 0)
    kbs = (kb0, kb1)

    def make_qm(q, nb, pos, hb):
        z8 = jnp.zeros((8, TQ), F32)
        if hb == 0:
            piece = [q[0:16], jnp.where(sub_q < 4, q[16:24], 0.0), z8, z8]
        else:
            piece = [z8, z8, jnp.where(sub_q >= 4, q[0:8], 0.0), q[8:24]]
        rows = []
        for pp in range(PPG):
            rows += [jnp.where(pos == pp, a, jnp.zeros_like(a)) for a in piece]
        rows.append(z8 if nb is None else jnp.where(sub_q == 0, nb, 0.0))
        return jnp.concatenate(rows, axis=0).astype(BF16)

    def v_lhs(r0, hb):
        sub = lax.broadcasted_iota(jnp.int32, (8, S), 0)
        v = vt_scr[pl.ds(r0 + 16 * hb, 24), :]
        if hb == 0:
            return jnp.concatenate([v[0:16], jnp.where(sub == 4, 1.0, v[16:24])], axis=0)
        return jnp.concatenate([jnp.where(sub == 3, 1.0, v[0:8]), v[8:24]], axis=0)

    LROW = (20, 3)

    def pair_setup(p):
        g = p // PPG
        return g, p - g * PPG, pl.multiple_of(p * PR, 8)

    def build_kb(p, hb, c):
        kx = kx_scr[p, XOFF[c]:XOFF[c] + XRS[c], :]
        for d in range(DH):
            col = hb * DH + d
            kbs[hb][d * XK + XOFF[c]:d * XK + XOFF[c] + XRS[c], :] = (
                jnp.broadcast_to(kx[:, col:col + 1], (XRS[c], 128)))

    def build_qh(p, hb, qi):
        for j in range(qi * CT, (qi + 1) * CT):
            cols = slice(j * 128, (j + 1) * 128)
            qh[j, 0:24, hb * 128:(hb + 1) * 128] = qt_scr[p, 16 * hb:16 * hb + 24, cols]
            qh[j, 24:32, hb * 128:(hb + 1) * 128] = qt_scr[p, PR:PR + 8, cols]

    def stage_x(rows):
        xst[...] = pltpu.bitcast(x_v[rows, :], U32)

    for c in range(NC):
        build_kb(0, 0, c)
    for qi in range(NQ):
        build_qh(0, 0, qi)
    stage_x(slice(0, FT))
    kst[...] = k_scr[0]

    def ffn_pieces(p, pn):
        rows = pl.ds(pl.multiple_of(p * FT, FT), FT)
        hs = []
        for n in range(DFF // 256):
            h = jnp.dot(pltpu.bitcast(xst[...], BF16), pltpu.bitcast(w1p[:, n * 256:(n + 1) * 256], BF16),
                        preferred_element_type=F32)
            hs.append(jnp.maximum(h, 0.0).astype(BF16))
            yield
        hh = jnp.concatenate(hs, axis=1)
        stage_x(pl.ds(pl.multiple_of(pn * FT, FT), FT))
        for n in range(D // 128):
            b_scr[rows, n * 128:(n + 1) * 128] = jnp.dot(
                hh, pltpu.bitcast(w2p[:, n * 128:(n + 1) * 128], BF16), preferred_element_type=F32)
            yield

    steps = [(hb, qi, c) for hb in range(2) for qi in range(NQ) for c in range(NC)]
    NS = len(steps)

    def fast_pair(p, carry):
        g, pos, r0 = pair_setup(p)
        pn = jnp.minimum(p + 1, NP - 1)
        hist = []

        def fence(hb):
            if not hist:
                return
            v = hist[-1]
            v = jnp.maximum(v[:, 0:8], v[:, 8:16])
            while v.shape[0] > 1:
                v = jnp.maximum(v[:v.shape[0] // 2], v[v.shape[0] // 2:])
            kbs[hb][kb_spare, :] = v[0]

        def vpu_block(hb, qi, row0):
            tiles = slice(qi * CT, (qi + 1) * CT)
            lanes = slice(hb * 128, (hb + 1) * 128)
            acc = None
            for d in range(DH):
                if d % G == 0:
                    fence(hb)
                if d == 0:
                    acc = jnp.broadcast_to(qh[tiles, 24 + hb:25 + hb, lanes], (CT, VB, 128))
                kb = kbs[hb][d * XK + row0:d * XK + row0 + VB, :]
                acc = acc + kb[None] * qh[tiles, 4 * hb + d:4 * hb + d + 1, lanes]
                if d % G == G - 1 - LK or d == DH - 1 - LK:
                    hist.append(acc)
            return jnp.concatenate([acc[c] for c in range(CT)], axis=1)

        @pl.when(jnp.logical_and(pos == 0, p > 0))
        def _():
            kst[...] = k_scr[g]

        for hb in range(2):
            vst[24 * hb:24 * hb + 24, :] = v_lhs(r0, hb)
        vst[v_spare, :] = jnp.zeros((8, S), F32)
        ffn = ffn_pieces(p, pn)
        next(ffn)
        ps, qms = {}, {}
        for t in range(NS + 1):
            if t < NS:
                hb, qi, c = steps[t]
                cols = slice(qi * TQ, (qi + 1) * TQ)
                if c == 0:
                    qms[(hb, qi)] = make_qm(qt_scr[p, 16 * hb:16 * hb + 24, cols],
                                            qt_scr[p, PR + hb:PR + hb + 1, cols], pos, hb)
                s = jnp.dot(pltpu.bitcast(kst[(c * TK + XRS[c]) // 2:(c + 1) * TK // 2, :], BF16),
                            qms[(hb, qi)], preferred_element_type=F32)
                sv = [vpu_block(hb, qi, XOFF[c] + b * VB) for b in range(XRS[c] // VB)]
                if (qi * NC + c) % NQ == 0:
                    build_kb(p if hb == 0 else pn, 1 - hb, (qi * NC + c) // NQ)
                if c == 0:
                    build_qh(p if hb == 0 else pn, 1 - hb, qi)
                s = jnp.concatenate(sv + [s], axis=0)
                ps[t] = jnp.exp2(jnp.concatenate(_to_keys(s, c), axis=0))
            if t >= 1:
                hb, qi, c = steps[t - 1]
                acc = jnp.dot(vst[24 * hb:24 * hb + 24, c * TK:(c + 1) * TK], ps.pop(t - 1),
                              preferred_element_type=F32)
                if c > 0:
                    acc = jnp.concatenate([accb[24 * j:24 * j + 24, :] for j in range(CT)], axis=1) + acc
                if c < NC - 1:
                    for j in range(CT):
                        accb[24 * j:24 * j + 24, :] = acc[:, 128 * j:128 * j + 128]
                    accb[acc_spare, :] = jnp.zeros((8, 128), F32)
                else:
                    cols = slice(qi * TQ, (qi + 1) * TQ)
                    ot_scr[p, 24 * hb:24 * hb + 24, cols] = acc
                    lmin_scr[:, cols] = jnp.minimum(lmin_scr[:, cols], acc[LROW[hb]:LROW[hb] + 1, :])
            if t % FFN_EVERY == 0:
                next(ffn, None)
        for _ in ffn:
            pass
        return carry

    lax.fori_loop(0, NP, fast_pair, 0)

    safe = jnp.logical_and(jnp.min(lmin_scr[...]) >= L_MIN, opaque0 == 0)

    @pl.when(jnp.logical_not(safe))
    def _():
        def slow_tile(it, carry):
            p = it // NQ
            qi = it - p * NQ
            g, pos, r0 = pair_setup(p)
            cols = pl.ds(pl.multiple_of(qi * TQ, TQ), TQ)
            for hb in range(2):
                qm = make_qm(qt_scr[p, 16 * hb:16 * hb + 24, cols], None, pos, hb)
                s = jnp.dot(pltpu.bitcast(k_scr[g], BF16), qm, preferred_element_type=F32)
                s = jnp.concatenate([a for c in range(NC) for a in _to_keys(s[c * TK:(c + 1) * TK], c)], axis=0)
                m = jnp.max(s, axis=0, keepdims=True)
                ot_scr[p, 24 * hb:24 * hb + 24, cols] = jnp.dot(
                    v_lhs(r0, hb), jnp.exp2(s - m), preferred_element_type=F32)
            return carry
        lax.fori_loop(0, NP * NQ, slow_tile, 0)

    def recip(l):
        r = pl.reciprocal(l, approx=True)
        return r * (2.0 - l * r)

    gw = gw_v[...].astype(F32).reshape(1, D)
    for i, (r0, r1) in enumerate(OUT_CHUNKS):
        rows = slice(r0, r1)
        sub = lax.broadcasted_iota(jnp.int32, (8, r1 - r0), 0)
        slabs = []
        for p in range(NP):
            oa = ot_scr[p, 0:24, rows]
            ob = ot_scr[p, 24:48, rows]
            oa = oa * recip(oa[LROW[0]:LROW[0] + 1, :])
            ob = ob * recip(ob[LROW[1]:LROW[1] + 1, :])
            slabs += [oa[0:16], jnp.where(sub < 4, oa[16:24], ob[0:8]), ob[8:24]]
        o = jnp.concatenate(slabs, axis=0).T.astype(BF16)
        a = jnp.dot(o, wo_v[...], preferred_element_type=F32)
        z = jnp.sum(x_v[rows, :].astype(F32) * gw, axis=1, keepdims=True)
        gt = 1.0 / (1.0 + jnp.exp(-z))
        o_v[rows, :] = (gt * a + (1.0 - gt) * b_scr[rows, :]).astype(o_v.dtype)
        cp_out[i].start()
    for cp in cp_out:
        cp.wait()


@jax.jit
def pallas_gated_mix__softmax_full_mha__dense_activation_relu__prompt_kernel(
        A_x, A_wqkv, A_wo, B_x, B_w1, B_w2, gate_w):
    return pl.pallas_call(
        _kernel,
        in_specs=[pl.BlockSpec(memory_space=pl.ANY)] * 6,
        out_specs=pl.BlockSpec(memory_space=pl.ANY),
        out_shape=jax.ShapeDtypeStruct((1, S, D), A_x.dtype),
        scratch_shapes=[
            pltpu.VMEM((S, D), BF16),
            pltpu.VMEM((D, 3 * D), BF16),
            pltpu.VMEM((D, D), BF16),
            pltpu.VMEM((D, DFF), BF16),
            pltpu.VMEM((DFF, D), BF16),
            pltpu.VMEM((D,), BF16),
            pltpu.VMEM((S, D), BF16),
            pltpu.VMEM((D // 2, NG * 128), U32),
            pltpu.VMEM((2 * D, D), BF16),
            pltpu.VMEM((NG, S // 2, 128), U32),
            pltpu.VMEM((NP, XK, 128), F32),
            pltpu.VMEM((NP, PR + 8, S), F32),
            pltpu.VMEM((D, S), F32),
            pltpu.VMEM((NP, 48, S), F32),
            pltpu.VMEM((1, S), F32),
            pltpu.VMEM((S, D), F32),
            pltpu.VMEM((DH * XK + 8, 128), F32),
            pltpu.VMEM((DH * XK + 8, 128), F32),
            pltpu.VMEM((S // 128, 32, 256), F32),
            pltpu.VMEM((S // 2, 128), U32),
            pltpu.VMEM((56, S), F32),
            pltpu.VMEM((FT // 2, D), U32),
            pltpu.VMEM((D // 2, DFF), U32),
            pltpu.VMEM((DFF // 2, D), U32),
            pltpu.VMEM((24 * CT + 8, 128), F32),
            pltpu.SemaphoreType.DMA((NSEM,)),
        ],
        compiler_params=pltpu.CompilerParams(vmem_limit_bytes=100 * 1024 * 1024),
    )(A_x, A_wqkv, A_wo, B_w1, B_w2, gate_w)
```

```python
import math
import jax
import jax.numpy as jnp
from jax import lax
import jax.experimental.pallas as pl
import jax.experimental.pallas.tpu as pltpu

S = 2048
D = 640
H = 32
DH = 20
DFF = 1536
NP = H // 2
PR = 2 * DH
PPG = 3
NG = 6
ONE_LANE = 120
TQ = 512
TK = 256
RC = 512
NRC = S // RC
NQ = S // TQ
NC = S // TK
CT = TQ // 128
FT = S // NP
QSCALE = (DH ** -0.5) * math.log2(math.e)
L_MIN = 2.0 ** -40
F32 = jnp.float32
BF16 = jnp.bfloat16
U32 = jnp.uint32
NT = (((1,), (1,)), ((), ()))

VB = 16
G = 7
LK = 2
FFN_EVERY = 4
XRS = [32] * (NC - 1) + [48]
XOFF = [sum(XRS[:c]) for c in range(NC)]
XK = sum(XRS)


def _stored_order(c):
    return list(range(XRS[c] // 8)) + list(range(TK // 8 - 1, XRS[c] // 8 - 1, -1))


def _to_stored(x, c):
    return [x[8 * j:8 * j + 8] for j in _stored_order(c)]


def _to_keys(x, c):
    o = _stored_order(c)
    return [x[8 * o.index(j):8 * o.index(j) + 8] for j in range(TK // 8)]


OUT_CHUNKS = [(0, 512), (512, 1024), (1024, 1536), (1536, 1920), (1920, 2048)]
NSEM = 12 + len(OUT_CHUNKS)
WAIT_R = 2


def _kernel(x_hbm, wqkv_hbm, wo_hbm, w1_hbm, w2_hbm, gw_hbm, o_hbm,
            x_v, wqkv_v, wo_v, w1_v, w2_v, gw_v, o_v,
            wkp_scr, wqvt_scr, k_scr, kx_scr, qt_scr, vt_scr, ot_scr, lmin_scr, b_scr,
            kb0, kb1, qh, kst, vst, xst, w1p, w2p, accb, sems):
    cp_wka = pltpu.make_async_copy(wqkv_hbm.at[:, D:D + 256], wqkv_v.at[:, D:D + 256], sems.at[0])
    cp_x = [pltpu.make_async_copy(x_hbm.at[0, r * RC:(r + 1) * RC, :], x_v.at[r * RC:(r + 1) * RC, :],
                                  sems.at[1 + r]) for r in range(NRC)]
    cp_wq = pltpu.make_async_copy(wqkv_hbm.at[:, 0:D], wqkv_v.at[:, 0:D], sems.at[5])
    cp_wv = pltpu.make_async_copy(wqkv_hbm.at[:, 2 * D:], wqkv_v.at[:, 2 * D:], sems.at[6])
    cp_w1 = pltpu.make_async_copy(w1_hbm, w1_v, sems.at[7])
    cp_w2 = pltpu.make_async_copy(w2_hbm, w2_v, sems.at[8])
    cp_wo = pltpu.make_async_copy(wo_hbm, wo_v, sems.at[9])
    cp_gw = pltpu.make_async_copy(gw_hbm, gw_v, sems.at[10])
    cp_wkb = pltpu.make_async_copy(wqkv_hbm.at[:, D + 256:2 * D], wqkv_v.at[:, D + 256:2 * D], sems.at[11])
    cp_out = [pltpu.make_async_copy(o_v.at[r0:r1, :], o_hbm.at[0, r0:r1, :], sems.at[12 + i])
              for i, (r0, r1) in enumerate(OUT_CHUNKS)]
    for cp in (cp_wka, cp_x[0], cp_wkb, cp_x[1], cp_x[2], cp_x[3], cp_wq, cp_wv, cp_w1, cp_w2, cp_wo, cp_gw):
        cp.start()

    GW = PPG * PR

    def regroup_wk(groups, c0, c1):
        for rb in range(D // 128):
            wk = pltpu.bitcast(wqkv_v[rb * 128:(rb + 1) * 128, D + c0:D + c1], U32)
            for g in groups:
                n = min(GW, D - g * GW)
                wkp_scr[rb * 64:(rb + 1) * 64, g * 128:(g + 1) * 128] = jnp.concatenate(
                    [wk[:, g * GW - c0:g * GW - c0 + n], jnp.zeros((64, 128 - n), U32)], axis=1)

    lane = lax.broadcasted_iota(jnp.int32, (RC, 128), 1)
    er = lax.broadcasted_iota(jnp.int32, (16, 128), 0)
    ec = lax.broadcasted_iota(jnp.int32, (16, 128), 1)
    e_k = jnp.where((ec >= er * DH) & (ec < er * DH + DH) & (er < 2 * PPG), 1.0, 0.0).astype(BF16)
    kn_max = [None] * NG

    def k_norm(r, g):
        kf = pltpu.bitcast(k_scr[g, r * RC // 2:(r + 1) * RC // 2, :], BF16).astype(F32)
        kn = lax.dot_general(e_k, (kf * kf).astype(BF16), NT, preferred_element_type=F32)[0:8]
        kn_max[g] = kn if kn_max[g] is None else jnp.maximum(kn_max[g], kn)

    def k_store(r, g, kg):
        k1 = jnp.where(lane == ONE_LANE, 1.0, kg)
        k1 = jnp.concatenate(
            [a for c in range(r * RC // TK, (r + 1) * RC // TK)
             for a in _to_stored(k1[c * TK - r * RC:(c + 1) * TK - r * RC], c)], axis=0)
        k_scr[g, r * RC // 2:(r + 1) * RC // 2, :] = pltpu.bitcast(k1.astype(BF16), U32)
        for c in range(r * RC // TK, (r + 1) * RC // TK):
            kx = k1[c * TK - r * RC:c * TK - r * RC + XRS[c]].astype(BF16).astype(F32)
            for pos in range(min(PPG, NP - g * PPG)):
                kx_scr[g * PPG + pos, XOFF[c]:XOFF[c] + XRS[c], :] = (
                    pltpu.roll(kx, 128 - pos * PR, axis=1) if pos else kx)

    def k_proj(r, pieces=((0, 1), (2, 3, 4))):
        xr = x_v[r * RC:(r + 1) * RC, :]
        for gs in pieces:
            w = pltpu.bitcast(wkp_scr[:, gs[0] * 128:(gs[-1] + 1) * 128], BF16)
            if len(pieces) == 1:
                ns = 2 if len(gs) == 2 else 4
                k = jnp.concatenate([jnp.dot(xr[i * RC // ns:(i + 1) * RC // ns], w, preferred_element_type=F32)
                                     for i in range(ns)], axis=0)
            else:
                k = jnp.dot(xr, w, preferred_element_type=F32)
            for g in gs:
                k_store(r, g, k[:, (g - gs[0]) * 128:(g - gs[0] + 1) * 128])
                if r > 0:
                    k_norm(r - 1, g)

    cp_wka.wait()
    cp_x[0].wait()
    regroup_wk((0, 1), 0, 256)
    k_proj(0, ((0, 1),))
    cp_wkb.wait()
    regroup_wk((2, 3, 4), 128, D)
    k_proj(0, ((2, 3, 4),))
    cp_x[1].wait()
    cp_x[2].wait()
    k_proj(1)
    k_proj(2)
    for cp in (cp_x[3], cp_wv, cp_wq):
        cp.wait()
    VT0 = D + 48
    for cb in range(D // 128):
        wqvt_scr[cb * 128:(cb + 1) * 128, :] = (
            wqkv_v[:, cb * 128:(cb + 1) * 128].astype(F32).T.astype(BF16))
    wqvt_scr[D:VT0, :] = wqkv_v[:, 2 * D - 128:2 * D].astype(F32).T[80:128].astype(BF16)
    for cb in range(D // 128):
        wqvt_scr[VT0 + cb * 128:VT0 + (cb + 1) * 128, :] = (
            wqkv_v[:, 2 * D + cb * 128:2 * D + (cb + 1) * 128].astype(F32).T.astype(BF16))
    k_proj(3)

    for r in range(NRC):
        if r == WAIT_R:
            for cp in (cp_w1, cp_w2, cp_wo, cp_gw):
                cp.wait()
            for rb in range(D // 128):
                w1p[rb * 64:(rb + 1) * 64, :] = pltpu.bitcast(w1_v[rb * 128:(rb + 1) * 128, :], U32)
            for rb in range(DFF // 128):
                w2p[rb * 64:(rb + 1) * 64, :] = pltpu.bitcast(w2_v[rb * 128:(rb + 1) * 128, :], U32)
        xr = x_v[r * RC:(r + 1) * RC, :]
        cols = slice(r * RC, (r + 1) * RC)
        for half in range(2):
            y = lax.dot_general(wqvt_scr[half * (D // 2):(D // 2 if half == 0 else VT0), :], xr, NT,
                                preferred_element_type=F32)
            q = (y[0:D // 2] * QSCALE).astype(BF16).astype(F32)
            for p in range(NP // 2):
                qt_scr[half * NP // 2 + p, 0:PR, cols] = q[p * PR:(p + 1) * PR]
            if 2 * r + half < NG - 1:
                k_norm(NRC - 1, 2 * r + half)
        kt = jnp.concatenate([y[D // 2 + 8:], jnp.zeros((128 - PR, RC), F32)], axis=0)
        k_store(r, NG - 1, kt.T)
        kk = kt[0:PR].astype(BF16).astype(F32)
        kk = kk * kk
        kn = jnp.concatenate([jnp.sum(kk[0:DH], axis=0, keepdims=True),
                              jnp.sum(kk[DH:PR], axis=0, keepdims=True)], axis=0)
        kn_max[NG - 1] = kn if r == 0 else jnp.maximum(kn_max[NG - 1], kn)
    kn_rows = [jnp.max(kn_max[g], axis=1, keepdims=True) for g in range(NG)]
    kn_col = jnp.concatenate([kn_rows[g][0:min(2 * PPG, H - 2 * PPG * g)] for g in range(NG)], axis=0)
    er = lax.broadcasted_iota(jnp.int32, (H, D), 0)
    ec = lax.broadcasted_iota(jnp.int32, (H, D), 1)
    e_q = jnp.where((ec >= er * DH) & (ec < er * DH + DH), 1.0, 0.0).astype(BF16)

    opaque0 = jnp.clip(-(jnp.minimum(jnp.min(kn_col), 0.0).astype(jnp.int32)), 0, DH * XK // 8)

    def spare(n):
        return pl.ds(pl.multiple_of((n - jnp.minimum(opaque0, n)) * 8, 8), 8)

    v_spare, acc_spare = spare(6), spare(3 * CT)
    kb_spare = (DH - jnp.minimum(opaque0, DH), spare(XK // 8 - 1), slice(None))

    def q_shift(cols):
        q = jnp.concatenate([qt_scr[p, 0:PR, cols] for p in range(NP)], axis=0)
        qn = jnp.dot(e_q, (q * q).astype(BF16), preferred_element_type=F32)
        nb = -(jnp.sqrt(qn * kn_col) * 1.02)
        nb = nb.astype(BF16).astype(F32)
        for p in range(NP):
            nbt = nb[8 * (p // 4):8 * (p // 4) + 8]
            if p % 4:
                nbt = pltpu.roll(nbt, 8 - 2 * (p % 4), axis=0)
            qt_scr[p, PR:PR + 8, cols] = nbt

    for r in range(NRC):
        xr = x_v[r * RC:(r + 1) * RC, :]
        cols = slice(r * RC, (r + 1) * RC)
        for half in range(2):
            rows = slice(half * (D // 2), (half + 1) * (D // 2))
            v = lax.dot_general(wqvt_scr[VT0 + rows.start:VT0 + rows.stop, :], xr, NT,
                                preferred_element_type=F32)
            vt_scr[rows, cols] = v.astype(BF16).astype(F32)
            if 2 * r + half < NRC:
                q_shift(slice((2 * r + half) * RC, (2 * r + half + 1) * RC))
    lmin_scr[...] = jnp.full(lmin_scr.shape, jnp.inf, F32)

    sub_q = lax.broadcasted_iota(jnp.int32, (8, TQ), 0)
    kbs = (kb0, kb1)

    def make_qm(q, nb, pos, hb):
        z8 = jnp.zeros((8, TQ), F32)
        if hb == 0:
            piece = [q[0:16], jnp.where(sub_q < 4, q[16:24], 0.0), z8, z8]
        else:
            piece = [z8, z8, jnp.where(sub_q >= 4, q[0:8], 0.0), q[8:24]]
        rows = []
        for pp in range(PPG):
            rows += [jnp.where(pos == pp, a, jnp.zeros_like(a)) for a in piece]
        rows.append(z8 if nb is None else jnp.where(sub_q == 0, nb, 0.0))
        return jnp.concatenate(rows, axis=0).astype(BF16)

    def v_lhs(r0, hb):
        sub = lax.broadcasted_iota(jnp.int32, (8, S), 0)
        v = vt_scr[pl.ds(r0 + 16 * hb, 24), :]
        if hb == 0:
            return jnp.concatenate([v[0:16], jnp.where(sub == 4, 1.0, v[16:24])], axis=0)
        return jnp.concatenate([jnp.where(sub == 3, 1.0, v[0:8]), v[8:24]], axis=0)

    LROW = (20, 3)

    def pair_setup(p):
        g = p // PPG
        return g, p - g * PPG, pl.multiple_of(p * PR, 8)

    def build_kb(p, hb, c):
        kx = kx_scr[p, XOFF[c]:XOFF[c] + XRS[c], :]
        kbs[hb][0:DH, XOFF[c]:XOFF[c] + XRS[c], :] = jnp.stack(
            [jnp.broadcast_to(kx[:, hb * DH + d:hb * DH + d + 1], (XRS[c], 128)) for d in range(DH)])

    def build_qh(p, hb, qi):
        for j in range(qi * CT, (qi + 1) * CT):
            cols = slice(j * 128, (j + 1) * 128)
            qh[j, 0:24, hb * 128:(hb + 1) * 128] = qt_scr[p, 16 * hb:16 * hb + 24, cols]
            qh[j, 24:32, hb * 128:(hb + 1) * 128] = qt_scr[p, PR:PR + 8, cols]

    def stage_x(rows):
        xst[...] = pltpu.bitcast(x_v[rows, :], U32)

    for c in range(NC):
        build_kb(0, 0, c)
    for qi in range(NQ):
        build_qh(0, 0, qi)
    stage_x(slice(0, FT))
    kst[...] = k_scr[0]

    def ffn_pieces(p, pn):
        rows = pl.ds(pl.multiple_of(p * FT, FT), FT)
        hs = []
        for n in range(DFF // 256):
            h = jnp.dot(pltpu.bitcast(xst[...], BF16), pltpu.bitcast(w1p[:, n * 256:(n + 1) * 256], BF16),
                        preferred_element_type=F32)
            hs.append(jnp.maximum(h, 0.0).astype(BF16))
            yield
        hh = jnp.concatenate(hs, axis=1)
        stage_x(pl.ds(pl.multiple_of(pn * FT, FT), FT))
        for n in range(D // 128):
            b_scr[rows, n * 128:(n + 1) * 128] = jnp.dot(
                hh, pltpu.bitcast(w2p[:, n * 128:(n + 1) * 128], BF16), preferred_element_type=F32)
            yield

    steps = [(hb, qi, c) for hb in range(2) for qi in range(NQ) for c in range(NC)]
    NS = len(steps)

    def fast_pair(p, carry):
        g, pos, r0 = pair_setup(p)
        pn = jnp.minimum(p + 1, NP - 1)
        hist = []

        def fence(hb):
            if not hist:
                return
            v = hist[-1]
            v = jnp.maximum(v[:, 0:8], v[:, 8:16])
            while v.shape[0] > 1:
                v = jnp.maximum(v[:v.shape[0] // 2], v[v.shape[0] // 2:])
            kbs[hb][kb_spare] = v[0]

        def vpu_block(hb, qi, row0):
            tiles = slice(qi * CT, (qi + 1) * CT)
            lanes = slice(hb * 128, (hb + 1) * 128)
            acc = None
            for d in range(DH):
                if d % G == 0:
                    fence(hb)
                    kbg = kbs[hb][d:min(d + G, DH), row0:row0 + VB, :]
                if d == 0:
                    acc = jnp.broadcast_to(qh[tiles, 24 + hb:25 + hb, lanes], (CT, VB, 128))
                acc = acc + kbg[d % G:d % G + 1] * qh[tiles, 4 * hb + d:4 * hb + d + 1, lanes]
                if d % G == G - 1 - LK or d == DH - 1 - LK:
                    hist.append(acc)
            return jnp.concatenate([acc[c] for c in range(CT)], axis=1)

        @pl.when(jnp.logical_and(pos == 0, p > 0))
        def _():
            kst[...] = k_scr[g]

        for hb in range(2):
            vst[24 * hb:24 * hb + 24, :] = v_lhs(r0, hb)
        vst[v_spare, :] = jnp.zeros((8, S), F32)
        ffn = ffn_pieces(p, pn)
        next(ffn)
        ps, qms = {}, {}
        for t in range(NS + 1):
            if t < NS:
                hb, qi, c = steps[t]
                cols = slice(qi * TQ, (qi + 1) * TQ)
                if c == 0:
                    qms[(hb, qi)] = make_qm(qt_scr[p, 16 * hb:16 * hb + 24, cols],
                                            qt_scr[p, PR + hb:PR + hb + 1, cols], pos, hb)
                s = jnp.dot(pltpu.bitcast(kst[(c * TK + XRS[c]) // 2:(c + 1) * TK // 2, :], BF16),
                            qms[(hb, qi)], preferred_element_type=F32)
                sv = [vpu_block(hb, qi, XOFF[c] + b * VB) for b in range(XRS[c] // VB)]
                if (qi * NC + c) % NQ == 0:
                    build_kb(p if hb == 0 else pn, 1 - hb, (qi * NC + c) // NQ)
                if c == 0:
                    build_qh(p if hb == 0 else pn, 1 - hb, qi)
                s = jnp.concatenate(sv + [s], axis=0)
                ps[t] = jnp.exp2(jnp.concatenate(_to_keys(s, c), axis=0))
            if t >= 1:
                hb, qi, c = steps[t - 1]
                acc = jnp.dot(vst[24 * hb:24 * hb + 24, c * TK:(c + 1) * TK], ps.pop(t - 1),
                              preferred_element_type=F32)
                if c > 0:
                    acc = jnp.concatenate([accb[24 * j:24 * j + 24, :] for j in range(CT)], axis=1) + acc
                if c < NC - 1:
                    for j in range(CT):
                        accb[24 * j:24 * j + 24, :] = acc[:, 128 * j:128 * j + 128]
                    accb[acc_spare, :] = jnp.zeros((8, 128), F32)
                else:
                    cols = slice(qi * TQ, (qi + 1) * TQ)
                    ot_scr[p, 24 * hb:24 * hb + 24, cols] = acc
                    lmin_scr[:, cols] = jnp.minimum(lmin_scr[:, cols], acc[LROW[hb]:LROW[hb] + 1, :])
            if t % FFN_EVERY == 0:
                next(ffn, None)
        for _ in ffn:
            pass
        return carry

    lax.fori_loop(0, NP, fast_pair, 0)

    safe = jnp.logical_and(jnp.min(lmin_scr[...]) >= L_MIN, opaque0 == 0)

    @pl.when(jnp.logical_not(safe))
    def _():
        def slow_tile(it, carry):
            p = it // NQ
            qi = it - p * NQ
            g, pos, r0 = pair_setup(p)
            cols = pl.ds(pl.multiple_of(qi * TQ, TQ), TQ)
            for hb in range(2):
                qm = make_qm(qt_scr[p, 16 * hb:16 * hb + 24, cols], None, pos, hb)
                s = jnp.dot(pltpu.bitcast(k_scr[g], BF16), qm, preferred_element_type=F32)
                s = jnp.concatenate([a for c in range(NC) for a in _to_keys(s[c * TK:(c + 1) * TK], c)], axis=0)
                m = jnp.max(s, axis=0, keepdims=True)
                ot_scr[p, 24 * hb:24 * hb + 24, cols] = jnp.dot(
                    v_lhs(r0, hb), jnp.exp2(s - m), preferred_element_type=F32)
            return carry
        lax.fori_loop(0, NP * NQ, slow_tile, 0)

    def recip(l):
        r = pl.reciprocal(l, approx=True)
        return r * (2.0 - l * r)

    gw = gw_v[...].astype(F32).reshape(1, D)
    for i, (r0, r1) in enumerate(OUT_CHUNKS):
        rows = slice(r0, r1)
        sub = lax.broadcasted_iota(jnp.int32, (8, r1 - r0), 0)
        slabs = []
        for p in range(NP):
            oa = ot_scr[p, 0:24, rows]
            ob = ot_scr[p, 24:48, rows]
            oa = oa * recip(oa[LROW[0]:LROW[0] + 1, :])
            ob = ob * recip(ob[LROW[1]:LROW[1] + 1, :])
            slabs += [oa[0:16], jnp.where(sub < 4, oa[16:24], ob[0:8]), ob[8:24]]
        o = jnp.concatenate(slabs, axis=0).T.astype(BF16)
        a = jnp.dot(o, wo_v[...], preferred_element_type=F32)
        z = jnp.sum(x_v[rows, :].astype(F32) * gw, axis=1, keepdims=True)
        gt = 1.0 / (1.0 + jnp.exp(-z))
        o_v[rows, :] = (gt * a + (1.0 - gt) * b_scr[rows, :]).astype(o_v.dtype)
        cp_out[i].start()
    for cp in cp_out:
        cp.wait()


@jax.jit
def pallas_gated_mix__softmax_full_mha__dense_activation_relu__prompt_kernel(
        A_x, A_wqkv, A_wo, B_x, B_w1, B_w2, gate_w):
    return pl.pallas_call(
        _kernel,
        in_specs=[pl.BlockSpec(memory_space=pl.ANY)] * 6,
        out_specs=pl.BlockSpec(memory_space=pl.ANY),
        out_shape=jax.ShapeDtypeStruct((1, S, D), A_x.dtype),
        scratch_shapes=[
            pltpu.VMEM((S, D), BF16),
            pltpu.VMEM((D, 3 * D), BF16),
            pltpu.VMEM((D, D), BF16),
            pltpu.VMEM((D, DFF), BF16),
            pltpu.VMEM((DFF, D), BF16),
            pltpu.VMEM((D,), BF16),
            pltpu.VMEM((S, D), BF16),
            pltpu.VMEM((D // 2, (NG - 1) * 128), U32),
            pltpu.VMEM((2 * D + 48, D), BF16),
            pltpu.VMEM((NG, S // 2, 128), U32),
            pltpu.VMEM((NP, XK, 128), F32),
            pltpu.VMEM((NP, PR + 8, S), F32),
            pltpu.VMEM((D, S), F32),
            pltpu.VMEM((NP, 48, S), F32),
            pltpu.VMEM((1, S), F32),
            pltpu.VMEM((S, D), F32),
            pltpu.VMEM((DH + 1, XK, 128), F32),
            pltpu.VMEM((DH + 1, XK, 128), F32),
            pltpu.VMEM((S // 128, 32, 256), F32),
            pltpu.VMEM((S // 2, 128), U32),
            pltpu.VMEM((56, S), F32),
            pltpu.VMEM((FT // 2, D), U32),
            pltpu.VMEM((D // 2, DFF), U32),
            pltpu.VMEM((DFF // 2, D), U32),
            pltpu.VMEM((24 * CT + 8, 128), F32),
            pltpu.SemaphoreType.DMA((NSEM,)),
        ],
        compiler_params=pltpu.CompilerParams(vmem_limit_bytes=100 * 1024 * 1024),
    )(A_x, A_wqkv, A_wo, B_w1, B_w2, gate_w)
```

```python
import math
import jax
import jax.numpy as jnp
from jax import lax
import jax.experimental.pallas as pl
import jax.experimental.pallas.tpu as pltpu

S = 2048
D = 640
H = 32
DH = 20
DFF = 1536
NP = H // 2
PR = 2 * DH
PPG = 3
NG = 6
ONE_LANE = 120
TQ = 512
TK = 256
RC = 512
NRC = S // RC
NQ = S // TQ
NC = S // TK
CT = TQ // 128
FT = S // NP
QSCALE = (DH ** -0.5) * math.log2(math.e)
L_MIN = 2.0 ** -40
F32 = jnp.float32
BF16 = jnp.bfloat16
U32 = jnp.uint32
NT = (((1,), (1,)), ((), ()))

VB = 16
G = 7
LK = 2
FFN_EVERY = 4
XRS = [32] * (NC - 1) + [48]
XOFF = [sum(XRS[:c]) for c in range(NC)]
XK = sum(XRS)


def _stored_order(c):
    return list(range(XRS[c] // 8)) + list(range(TK // 8 - 1, XRS[c] // 8 - 1, -1))


def _to_stored(x, c):
    return [x[8 * j:8 * j + 8] for j in _stored_order(c)]


def _to_keys(x, c):
    o = _stored_order(c)
    return [x[8 * o.index(j):8 * o.index(j) + 8] for j in range(TK // 8)]


OUT_CHUNKS = [(0, 512), (512, 1024), (1024, 1536), (1536, 1920), (1920, 2048)]
NSEM = 12 + len(OUT_CHUNKS)
WAIT_R = 2


def _kernel(x_hbm, wqkv_hbm, wo_hbm, w1_hbm, w2_hbm, gw_hbm, o_hbm,
            x_v, wqkv_v, wo_v, w1_v, w2_v, gw_v, o_v,
            wkp_scr, wqvt_scr, k_scr, kx_scr, qt_scr, vt_scr, ot_scr, lmin_scr, b_scr,
            kb0, kb1, qh, kst, vst, xst, w1p, w2p, accb, sems):
    cp_wka = pltpu.make_async_copy(wqkv_hbm.at[:, D:D + 256], wqkv_v.at[:, D:D + 256], sems.at[0])
    cp_x = [pltpu.make_async_copy(x_hbm.at[0, r * RC:(r + 1) * RC, :], x_v.at[r * RC:(r + 1) * RC, :],
                                  sems.at[1 + r]) for r in range(NRC)]
    cp_wq = pltpu.make_async_copy(wqkv_hbm.at[:, 0:D], wqkv_v.at[:, 0:D], sems.at[5])
    cp_wv = pltpu.make_async_copy(wqkv_hbm.at[:, 2 * D:], wqkv_v.at[:, 2 * D:], sems.at[6])
    cp_w1 = pltpu.make_async_copy(w1_hbm, w1_v, sems.at[7])
    cp_w2 = pltpu.make_async_copy(w2_hbm, w2_v, sems.at[8])
    cp_wo = pltpu.make_async_copy(wo_hbm, wo_v, sems.at[9])
    cp_gw = pltpu.make_async_copy(gw_hbm, gw_v, sems.at[10])
    cp_wkb = pltpu.make_async_copy(wqkv_hbm.at[:, D + 256:2 * D], wqkv_v.at[:, D + 256:2 * D], sems.at[11])
    cp_out = [pltpu.make_async_copy(o_v.at[r0:r1, :], o_hbm.at[0, r0:r1, :], sems.at[12 + i])
              for i, (r0, r1) in enumerate(OUT_CHUNKS)]
    for cp in (cp_wka, cp_x[0], cp_wkb, cp_x[1], cp_x[2], cp_x[3], cp_wq, cp_wv, cp_w1, cp_w2, cp_wo, cp_gw):
        cp.start()

    GW = PPG * PR

    def regroup_wk(groups, c0, c1):
        for rb in range(D // 128):
            wk = pltpu.bitcast(wqkv_v[rb * 128:(rb + 1) * 128, D + c0:D + c1], U32)
            for g in groups:
                n = min(GW, D - g * GW)
                wkp_scr[rb * 64:(rb + 1) * 64, g * 128:(g + 1) * 128] = jnp.concatenate(
                    [wk[:, g * GW - c0:g * GW - c0 + n], jnp.zeros((64, 128 - n), U32)], axis=1)

    lane = lax.broadcasted_iota(jnp.int32, (RC, 128), 1)
    er = lax.broadcasted_iota(jnp.int32, (16, 128), 0)
    ec = lax.broadcasted_iota(jnp.int32, (16, 128), 1)
    e_k = jnp.where((ec >= er * DH) & (ec < er * DH + DH) & (er < 2 * PPG), 1.0, 0.0).astype(BF16)
    kn_max = [None] * NG

    def k_norm(r, g):
        kf = pltpu.bitcast(k_scr[g, r * RC // 2:(r + 1) * RC // 2, :], BF16).astype(F32)
        kn = lax.dot_general(e_k, (kf * kf).astype(BF16), NT, preferred_element_type=F32)[0:8]
        kn_max[g] = kn if kn_max[g] is None else jnp.maximum(kn_max[g], kn)

    def k_store(r, g, kg):
        k1 = jnp.where(lane == ONE_LANE, 1.0, kg)
        k1 = jnp.concatenate(
            [a for c in range(r * RC // TK, (r + 1) * RC // TK)
             for a in _to_stored(k1[c * TK - r * RC:(c + 1) * TK - r * RC], c)], axis=0)
        k_scr[g, r * RC // 2:(r + 1) * RC // 2, :] = pltpu.bitcast(k1.astype(BF16), U32)
        for c in range(r * RC // TK, (r + 1) * RC // TK):
            kx = k1[c * TK - r * RC:c * TK - r * RC + XRS[c]].astype(BF16).astype(F32)
            for pos in range(min(PPG, NP - g * PPG)):
                kx_scr[g * PPG + pos, XOFF[c]:XOFF[c] + XRS[c], :] = (
                    pltpu.roll(kx, 128 - pos * PR, axis=1) if pos else kx)

    def k_proj(r, pieces=((0, 1), (2, 3, 4))):
        xr = x_v[r * RC:(r + 1) * RC, :]
        for gs in pieces:
            w = pltpu.bitcast(wkp_scr[:, gs[0] * 128:(gs[-1] + 1) * 128], BF16)
            if len(pieces) == 1:
                ns = 2 if len(gs) == 2 else 4
                k = jnp.concatenate([jnp.dot(xr[i * RC // ns:(i + 1) * RC // ns], w, preferred_element_type=F32)
                                     for i in range(ns)], axis=0)
            else:
                k = jnp.dot(xr, w, preferred_element_type=F32)
            for g in gs:
                k_store(r, g, k[:, (g - gs[0]) * 128:(g - gs[0] + 1) * 128])
                if r > 0:
                    k_norm(r - 1, g)

    cp_wka.wait()
    cp_x[0].wait()
    regroup_wk((0, 1), 0, 256)
    k_proj(0, ((0, 1),))
    cp_wkb.wait()
    regroup_wk((2, 3, 4), 128, D)
    k_proj(0, ((2, 3, 4),))
    cp_x[1].wait()
    k_proj(1, ((0, 1, 2, 3, 4),))
    for cp in (cp_x[2], cp_x[3], cp_wq):
        cp.wait()
    VT0 = D + 48
    for cb in range(D // 128):
        wqvt_scr[cb * 128:(cb + 1) * 128, :] = (
            wqkv_v[:, cb * 128:(cb + 1) * 128].astype(F32).T.astype(BF16))
    wqvt_scr[D:VT0, :] = wqkv_v[:, 2 * D - 128:2 * D].astype(F32).T[80:128].astype(BF16)
    k_proj(2)
    k_proj(3)

    for r in range(NRC):
        if r == WAIT_R:
            for cp in (cp_wv, cp_w1, cp_w2):
                cp.wait()
            for cb in range(D // 128):
                wqvt_scr[VT0 + cb * 128:VT0 + (cb + 1) * 128, :] = (
                    wqkv_v[:, 2 * D + cb * 128:2 * D + (cb + 1) * 128].astype(F32).T.astype(BF16))
            for rb in range(D // 128):
                w1p[rb * 64:(rb + 1) * 64, :] = pltpu.bitcast(w1_v[rb * 128:(rb + 1) * 128, :], U32)
            for rb in range(DFF // 128):
                w2p[rb * 64:(rb + 1) * 64, :] = pltpu.bitcast(w2_v[rb * 128:(rb + 1) * 128, :], U32)
        xr = x_v[r * RC:(r + 1) * RC, :]
        cols = slice(r * RC, (r + 1) * RC)
        for half in range(2):
            y = lax.dot_general(wqvt_scr[half * (D // 2):(D // 2 if half == 0 else VT0), :], xr, NT,
                                preferred_element_type=F32)
            q = (y[0:D // 2] * QSCALE).astype(BF16).astype(F32)
            for p in range(NP // 2):
                qt_scr[half * NP // 2 + p, 0:PR, cols] = q[p * PR:(p + 1) * PR]
            if 2 * r + half < NG - 1:
                k_norm(NRC - 1, 2 * r + half)
        kt = jnp.concatenate([y[D // 2 + 8:], jnp.zeros((128 - PR, RC), F32)], axis=0)
        k_store(r, NG - 1, kt.T)
        kk = kt[0:PR].astype(BF16).astype(F32)
        kk = kk * kk
        kn = jnp.concatenate([jnp.sum(kk[0:DH], axis=0, keepdims=True),
                              jnp.sum(kk[DH:PR], axis=0, keepdims=True)], axis=0)
        kn_max[NG - 1] = kn if r == 0 else jnp.maximum(kn_max[NG - 1], kn)
    kn_rows = [jnp.max(kn_max[g], axis=1, keepdims=True) for g in range(NG)]
    kn_col = jnp.concatenate([kn_rows[g][0:min(2 * PPG, H - 2 * PPG * g)] for g in range(NG)], axis=0)
    er = lax.broadcasted_iota(jnp.int32, (H, D), 0)
    ec = lax.broadcasted_iota(jnp.int32, (H, D), 1)
    e_q = jnp.where((ec >= er * DH) & (ec < er * DH + DH), 1.0, 0.0).astype(BF16)

    opaque0 = jnp.clip(-(jnp.minimum(jnp.min(kn_col), 0.0).astype(jnp.int32)), 0, DH * XK // 8)

    def spare(n):
        return pl.ds(pl.multiple_of((n - jnp.minimum(opaque0, n)) * 8, 8), 8)

    v_spare, acc_spare = spare(6), spare(3 * CT)
    kb_spare = (DH - jnp.minimum(opaque0, DH), spare(XK // 8 - 1), slice(None))

    def q_shift(cols):
        q = jnp.concatenate([qt_scr[p, 0:PR, cols] for p in range(NP)], axis=0)
        qn = jnp.dot(e_q, (q * q).astype(BF16), preferred_element_type=F32)
        nb = -(jnp.sqrt(qn * kn_col) * 1.02)
        nb = nb.astype(BF16).astype(F32)
        for p in range(NP):
            nbt = nb[8 * (p // 4):8 * (p // 4) + 8]
            if p % 4:
                nbt = pltpu.roll(nbt, 8 - 2 * (p % 4), axis=0)
            qt_scr[p, PR:PR + 8, cols] = nbt

    for r in range(NRC):
        xr = x_v[r * RC:(r + 1) * RC, :]
        cols = slice(r * RC, (r + 1) * RC)
        for half in range(2):
            rows = slice(half * (D // 2), (half + 1) * (D // 2))
            v = lax.dot_general(wqvt_scr[VT0 + rows.start:VT0 + rows.stop, :], xr, NT,
                                preferred_element_type=F32)
            vt_scr[rows, cols] = v.astype(BF16).astype(F32)
            if 2 * r + half < NRC:
                q_shift(slice((2 * r + half) * RC, (2 * r + half + 1) * RC))
    lmin_scr[...] = jnp.full(lmin_scr.shape, jnp.inf, F32)

    sub_q = lax.broadcasted_iota(jnp.int32, (8, TQ), 0)
    kbs = (kb0, kb1)

    def make_qm(q, nb, pos, hb):
        z8 = jnp.zeros((8, TQ), F32)
        if hb == 0:
            piece = [q[0:16], jnp.where(sub_q < 4, q[16:24], 0.0), z8, z8]
        else:
            piece = [z8, z8, jnp.where(sub_q >= 4, q[0:8], 0.0), q[8:24]]
        rows = []
        for pp in range(PPG):
            rows += [jnp.where(pos == pp, a, jnp.zeros_like(a)) for a in piece]
        rows.append(z8 if nb is None else jnp.where(sub_q == 0, nb, 0.0))
        return jnp.concatenate(rows, axis=0).astype(BF16)

    def v_lhs(r0, hb):
        sub = lax.broadcasted_iota(jnp.int32, (8, S), 0)
        v = vt_scr[pl.ds(r0 + 16 * hb, 24), :]
        if hb == 0:
            return jnp.concatenate([v[0:16], jnp.where(sub == 4, 1.0, v[16:24])], axis=0)
        return jnp.concatenate([jnp.where(sub == 3, 1.0, v[0:8]), v[8:24]], axis=0)

    LROW = (20, 3)

    def pair_setup(p):
        g = p // PPG
        return g, p - g * PPG, pl.multiple_of(p * PR, 8)

    def build_kb(p, hb, c):
        kx = kx_scr[p, XOFF[c]:XOFF[c] + XRS[c], :]
        kbs[hb][0:DH, XOFF[c]:XOFF[c] + XRS[c], :] = jnp.stack(
            [jnp.broadcast_to(kx[:, hb * DH + d:hb * DH + d + 1], (XRS[c], 128)) for d in range(DH)])

    def build_qh(p, hb, qi):
        for j in range(qi * CT, (qi + 1) * CT):
            cols = slice(j * 128, (j + 1) * 128)
            qh[j, 0:24, hb * 128:(hb + 1) * 128] = qt_scr[p, 16 * hb:16 * hb + 24, cols]
            qh[j, 24:32, hb * 128:(hb + 1) * 128] = qt_scr[p, PR:PR + 8, cols]

    def stage_x(rows):
        xst[...] = pltpu.bitcast(x_v[rows, :], U32)

    for c in range(NC):
        build_kb(0, 0, c)
    for qi in range(NQ):
        build_qh(0, 0, qi)
    stage_x(slice(0, FT))
    kst[...] = k_scr[0]

    def ffn_pieces(p, pn):
        rows = pl.ds(pl.multiple_of(p * FT, FT), FT)
        hs = []
        for n in range(DFF // 256):
            h = jnp.dot(pltpu.bitcast(xst[...], BF16), pltpu.bitcast(w1p[:, n * 256:(n + 1) * 256], BF16),
                        preferred_element_type=F32)
            hs.append(jnp.maximum(h, 0.0).astype(BF16))
            yield
        hh = jnp.concatenate(hs, axis=1)
        stage_x(pl.ds(pl.multiple_of(pn * FT, FT), FT))
        for n in range(D // 128):
            b_scr[rows, n * 128:(n + 1) * 128] = jnp.dot(
                hh, pltpu.bitcast(w2p[:, n * 128:(n + 1) * 128], BF16), preferred_element_type=F32)
            yield

    steps = [(hb, qi, c) for hb in range(2) for qi in range(NQ) for c in range(NC)]
    NS = len(steps)

    def fast_pair(p, carry):
        g, pos, r0 = pair_setup(p)
        pn = jnp.minimum(p + 1, NP - 1)
        hist = []

        def fence(hb):
            if not hist:
                return
            v = hist[-1]
            v = jnp.maximum(v[:, 0:8], v[:, 8:16])
            while v.shape[0] > 1:
                v = jnp.maximum(v[:v.shape[0] // 2], v[v.shape[0] // 2:])
            kbs[hb][kb_spare] = v[0]

        def vpu_block(hb, qi, row0):
            tiles = slice(qi * CT, (qi + 1) * CT)
            lanes = slice(hb * 128, (hb + 1) * 128)
            acc = None
            for d in range(DH):
                if d % G == 0:
                    fence(hb)
                    kbg = kbs[hb][d:min(d + G, DH), row0:row0 + VB, :]
                if d == 0:
                    acc = jnp.broadcast_to(qh[tiles, 24 + hb:25 + hb, lanes], (CT, VB, 128))
                acc = acc + kbg[d % G:d % G + 1] * qh[tiles, 4 * hb + d:4 * hb + d + 1, lanes]
                if d % G == G - 1 - LK or d == DH - 1 - LK:
                    hist.append(acc)
            return jnp.concatenate([acc[c] for c in range(CT)], axis=1)

        @pl.when(jnp.logical_and(pos == 0, p > 0))
        def _():
            kst[...] = k_scr[g]

        for hb in range(2):
            vst[24 * hb:24 * hb + 24, :] = v_lhs(r0, hb)
        vst[v_spare, :] = jnp.zeros((8, S), F32)
        ffn = ffn_pieces(p, pn)
        next(ffn)
        ps, qms = {}, {}
        for t in range(NS + 1):
            if t < NS:
                hb, qi, c = steps[t]
                cols = slice(qi * TQ, (qi + 1) * TQ)
                if c == 0:
                    qms[(hb, qi)] = make_qm(qt_scr[p, 16 * hb:16 * hb + 24, cols],
                                            qt_scr[p, PR + hb:PR + hb + 1, cols], pos, hb)
                s = jnp.dot(pltpu.bitcast(kst[(c * TK + XRS[c]) // 2:(c + 1) * TK // 2, :], BF16),
                            qms[(hb, qi)], preferred_element_type=F32)
                sv = [vpu_block(hb, qi, XOFF[c] + b * VB) for b in range(XRS[c] // VB)]
                if (qi * NC + c) % NQ == 0:
                    build_kb(p if hb == 0 else pn, 1 - hb, (qi * NC + c) // NQ)
                if c == 0:
                    build_qh(p if hb == 0 else pn, 1 - hb, qi)
                s = jnp.concatenate(sv + [s], axis=0)
                ps[t] = jnp.exp2(jnp.concatenate(_to_keys(s, c), axis=0))
            if t >= 1:
                hb, qi, c = steps[t - 1]
                acc = jnp.dot(vst[24 * hb:24 * hb + 24, c * TK:(c + 1) * TK], ps.pop(t - 1),
                              preferred_element_type=F32)
                if c > 0:
                    acc = jnp.concatenate([accb[24 * j:24 * j + 24, :] for j in range(CT)], axis=1) + acc
                if c < NC - 1:
                    for j in range(CT):
                        accb[24 * j:24 * j + 24, :] = acc[:, 128 * j:128 * j + 128]
                    accb[acc_spare, :] = jnp.zeros((8, 128), F32)
                else:
                    cols = slice(qi * TQ, (qi + 1) * TQ)
                    ot_scr[p, 24 * hb:24 * hb + 24, cols] = acc
                    lmin_scr[:, cols] = jnp.minimum(lmin_scr[:, cols], acc[LROW[hb]:LROW[hb] + 1, :])
            if t % FFN_EVERY == 0:
                next(ffn, None)
        for _ in ffn:
            pass
        return carry

    lax.fori_loop(0, NP, fast_pair, 0)

    safe = jnp.logical_and(jnp.min(lmin_scr[...]) >= L_MIN, opaque0 == 0)

    @pl.when(jnp.logical_not(safe))
    def _():
        def slow_tile(it, carry):
            p = it // NQ
            qi = it - p * NQ
            g, pos, r0 = pair_setup(p)
            cols = pl.ds(pl.multiple_of(qi * TQ, TQ), TQ)
            for hb in range(2):
                qm = make_qm(qt_scr[p, 16 * hb:16 * hb + 24, cols], None, pos, hb)
                s = jnp.dot(pltpu.bitcast(k_scr[g], BF16), qm, preferred_element_type=F32)
                s = jnp.concatenate([a for c in range(NC) for a in _to_keys(s[c * TK:(c + 1) * TK], c)], axis=0)
                m = jnp.max(s, axis=0, keepdims=True)
                ot_scr[p, 24 * hb:24 * hb + 24, cols] = jnp.dot(
                    v_lhs(r0, hb), jnp.exp2(s - m), preferred_element_type=F32)
            return carry
        lax.fori_loop(0, NP * NQ, slow_tile, 0)

    def recip(l):
        r = pl.reciprocal(l, approx=True)
        return r * (2.0 - l * r)

    cp_wo.wait()
    cp_gw.wait()
    gw = gw_v[...].astype(F32).reshape(1, D)
    for i, (r0, r1) in enumerate(OUT_CHUNKS):
        rows = slice(r0, r1)
        sub = lax.broadcasted_iota(jnp.int32, (8, r1 - r0), 0)
        slabs = []
        for p in range(NP):
            oa = ot_scr[p, 0:24, rows]
            ob = ot_scr[p, 24:48, rows]
            oa = oa * recip(oa[LROW[0]:LROW[0] + 1, :])
            ob = ob * recip(ob[LROW[1]:LROW[1] + 1, :])
            slabs += [oa[0:16], jnp.where(sub < 4, oa[16:24], ob[0:8]), ob[8:24]]
        o = jnp.concatenate(slabs, axis=0).T.astype(BF16)
        a = jnp.dot(o, wo_v[...], preferred_element_type=F32)
        z = jnp.sum(x_v[rows, :].astype(F32) * gw, axis=1, keepdims=True)
        gt = 1.0 / (1.0 + jnp.exp(-z))
        o_v[rows, :] = (gt * a + (1.0 - gt) * b_scr[rows, :]).astype(o_v.dtype)
        cp_out[i].start()
    for cp in cp_out:
        cp.wait()


@jax.jit
def pallas_gated_mix__softmax_full_mha__dense_activation_relu__prompt_kernel(
        A_x, A_wqkv, A_wo, B_x, B_w1, B_w2, gate_w):
    return pl.pallas_call(
        _kernel,
        in_specs=[pl.BlockSpec(memory_space=pl.ANY)] * 6,
        out_specs=pl.BlockSpec(memory_space=pl.ANY),
        out_shape=jax.ShapeDtypeStruct((1, S, D), A_x.dtype),
        scratch_shapes=[
            pltpu.VMEM((S, D), BF16),
            pltpu.VMEM((D, 3 * D), BF16),
            pltpu.VMEM((D, D), BF16),
            pltpu.VMEM((D, DFF), BF16),
            pltpu.VMEM((DFF, D), BF16),
            pltpu.VMEM((D,), BF16),
            pltpu.VMEM((S, D), BF16),
            pltpu.VMEM((D // 2, (NG - 1) * 128), U32),
            pltpu.VMEM((2 * D + 48, D), BF16),
            pltpu.VMEM((NG, S // 2, 128), U32),
            pltpu.VMEM((NP, XK, 128), F32),
            pltpu.VMEM((NP, PR + 8, S), F32),
            pltpu.VMEM((D, S), F32),
            pltpu.VMEM((NP, 48, S), F32),
            pltpu.VMEM((1, S), F32),
            pltpu.VMEM((S, D), F32),
            pltpu.VMEM((DH + 1, XK, 128), F32),
            pltpu.VMEM((DH + 1, XK, 128), F32),
            pltpu.VMEM((S // 128, 32, 256), F32),
            pltpu.VMEM((S // 2, 128), U32),
            pltpu.VMEM((56, S), F32),
            pltpu.VMEM((FT // 2, D), U32),
            pltpu.VMEM((D // 2, DFF), U32),
            pltpu.VMEM((DFF // 2, D), U32),
            pltpu.VMEM((24 * CT + 8, 128), F32),
            pltpu.SemaphoreType.DMA((NSEM,)),
        ],
        compiler_params=pltpu.CompilerParams(vmem_limit_bytes=100 * 1024 * 1024),
    )(A_x, A_wqkv, A_wo, B_w1, B_w2, gate_w)
```
